```python
import jax
import jax.numpy as jnp

def _softmax(x, axis=-1):
    return jax.nn.softmax(x, axis=axis)
def _gelu(x):
    return jax.nn.gelu(x, approximate=True)
def _silu(x):
    return jax.nn.silu(x)
def _sigmoid(x):
    return jax.nn.sigmoid(x)
def _layernorm(x, axis=-1, eps=1e-5):
    m = jnp.mean(x, axis=axis, keepdims=True)
    v = jnp.var(x, axis=axis, keepdims=True)
    return (x - m) / jnp.sqrt(v + eps)
def _scatter_add(tgt, idx, src, axis=0):
    return tgt.at[idx].add(src)
def _segment_sum(src, seg, n):
    return jax.ops.segment_sum(src, seg, n)
class _Rng:
    def __init__(self, key):
        self._k = key
    def _next(self):
        self._k, sub = jax.random.split(self._k)
        return sub
    def normal(self, shape):
        return jax.random.normal(self._next(), shape, dtype=jnp.bfloat16)
    def randint(self, lo, hi, shape):
        return jax.random.randint(self._next(), shape, lo, hi, dtype=jnp.int32)
    def uniform(self, shape, lo=0.0, hi=1.0):
        return jax.random.uniform(self._next(), shape, jnp.bfloat16, lo, hi)
    def permutation(self, n):
        return jax.random.permutation(self._next(), n)


kernel_name = 'concat_heads__linear_attn_block__ssm_conv_h3__prompt'

def setup_inputs():
    _rng = _Rng(jax.random.key(int.from_bytes(__import__("os").urandom(4), "little")))
    _w = (lambda a: (lambda t: t.astype(jnp.bfloat16) if jnp.issubdtype(t.dtype, jnp.floating) else t)(jnp.asarray(a)))
    def _A_setup():
        B, S, D = 1, 2048, 1024
        return {
            "x": _w((lambda *s: _rng.normal(s) * 0.05)(B, S, D)),
            "wqkv": _w((lambda *s: _rng.normal(s) * 0.05)(D, 3 * D)),
            "wo": _w((lambda *s: _rng.normal(s) * 0.05)(D, D)),
        }
    _A_in = _A_setup()

    def _B_setup():
        B, S, D = 1, 2048, 1024
        ks = 4
        return {
            "q": _w((lambda *s: _rng.normal(s) * 0.05)(B, S, D)),
            "k": _w((lambda *s: _rng.normal(s) * 0.05)(B, S, D)),
            "v": _w((lambda *s: _rng.normal(s) * 0.05)(B, S, D)),
            "shift_k": _w((lambda *s: _rng.normal(s) * 0.05)(D, ks) * 0.5),
            "ssm_k": _w((lambda *s: _rng.normal(s) * 0.05)(D, S) * (1.0 / S ** 0.5)),
            "ssm_D": _w((lambda *s: _rng.normal(s) * 0.05)(D)),
        }
    _B_in = _B_setup()

    return {
        "A_x": _A_in["x"],
        "A_wqkv": _A_in["wqkv"],
        "A_wo": _A_in["wo"],
        "B_q": _B_in["q"],
        "B_k": _B_in["k"],
        "B_v": _B_in["v"],
        "B_shift_k": _B_in["shift_k"],
        "B_ssm_k": _B_in["ssm_k"],
        "B_ssm_D": _B_in["ssm_D"],
    }

def reference(A_x, A_wqkv, A_wo, B_q, B_k, B_v, B_shift_k, B_ssm_k, B_ssm_D):
    def _A_ref(x, wqkv, wo):
        B, S, D = x.shape
        H = 32; Dh = D // H
        qkv = (lambda x, *d: x.transpose(*d))((x @ wqkv).reshape(B, S, 3, H, Dh), 2, 0, 3, 1, 4)
        q, k, v = qkv[0], qkv[1], qkv[2]
        phi = lambda t: jnp.where(t > 0, t + 1, jnp.exp(t)) + 1e-6
        pq, pk = phi(q), phi(k)
        kv = jnp.einsum("bhsd,bhse->bhde", pk, v)
        z = jnp.einsum("bhsd->bhd", pk)
        num = jnp.einsum("bhqd,bhde->bhqe", pq, kv)
        den = jnp.einsum("bhqd,bhd->bhq", pq, z)[..., None] + 1e-6
        o = num / den
        return (lambda x, *d: x.transpose(*d))(o, 0, 2, 1, 3).reshape(B, S, D) @ wo

    def _B_ref(q, k, v, shift_k, ssm_k, ssm_D):
        B, S, D = q.shape
        ks = shift_k.shape[-1]
        k_pad = jnp.pad(k, ((0, 0), (ks - 1, 0), (0, 0)))
        k_shift = jnp.zeros_like(k)
        for t in range(ks):
            k_shift = k_shift + k_pad[:, t:t + S, :] * shift_k[:, ks - 1 - t][None, None, :]
        kv = k_shift * v
        L = 2 * S
        kv_pad = jnp.pad(kv, ((0, 0), (0, S), (0, 0)))
        kf_pad = jnp.pad(ssm_k, ((0, 0), (0, S)))
        kv_f = (lambda x, axes=(-2,-1): jnp.fft.rfft2(x.astype(jnp.float32), axes=axes))(kv_pad[:, None, :, :], axes=(1, 2))
        kf_f = (lambda x, axes=(-2,-1): jnp.fft.rfft2(x.astype(jnp.float32), axes=axes))(kf_pad[:, None, :], axes=(1, 2))
        kf_f = (lambda x, *d: x.transpose(*d))(kf_f, 1, 2, 0)
        y_f = kv_f * kf_f[None, :, :, :]
        y = (lambda x, s, axes=(-2,-1): jnp.fft.irfft2(x, s=s, axes=axes).astype(jnp.bfloat16))(y_f, (1, L), axes=(1, 2))[:, 0, :S, :]
        y = y + kv * ssm_D[None, None, :]
        return q * y

    a = _A_ref(A_x, A_wqkv, A_wo)
    b = _B_ref(B_q, B_k, B_v, B_shift_k, B_ssm_k, B_ssm_D)
    return jnp.concatenate([a, b], axis=-1)
```

```python
import numpy as np
import jax
import jax.numpy as jnp
from jax import lax
from jax.experimental import pallas as pl
from jax.experimental.pallas import tpu as pltpu

S, D = 2048, 1024
C = 128
NT = D // C
MF = 1024
R = 256
NR = S // R
MA = 128
BF = jnp.bfloat16
F32 = jnp.float32
U32 = jnp.uint32

FWD_CH = 32
BACK_CH = 64


def _make_consts():
    p = np.arange(16)[:, None]
    s = np.arange(8)[None, :]
    k1 = np.where(p < 8, 2 * (8 * p + s), 2 * (8 * (p - 8) + s) + 1)
    t1 = np.arange(128)
    F = np.zeros((4, 256, 128), np.float64)
    for t2 in range(4):
        th = 2 * np.pi * (4 * t1[None, None, :] + t2) * (k1[:, :, None] + 0.5) / MF
        F[t2] = np.stack([np.cos(th), -np.sin(th)], axis=1).reshape(256, 128)
    Finv = np.transpose(F, (0, 2, 1)) * (2.0 / MF)
    return F.astype(np.float32), Finv.astype(np.float32)


def _pack_rows(a):
    a = np.ascontiguousarray(a, np.float32)
    u = a.view(np.uint32)
    b = ((u + 0x7FFF + ((u >> 16) & 1)) >> 16).astype(np.uint32)
    return (b[..., 0::2, :] | (b[..., 1::2, :] << 16)).astype(np.uint32)


_F_NP, _FINV_NP = _make_consts()
_F_PK = _pack_rows(_F_NP)
_FINV_PK = _pack_rows(_FINV_NP)


def _lo(w):
    return pltpu.bitcast(w << 16, F32)


def _hi(w):
    return pltpu.bitcast(w & jnp.uint32(0xFFFF0000), F32)


def _bf(w):
    return pltpu.bitcast(w, BF)


def _pk(v):
    return pltpu.bitcast(v.astype(BF), U32)


def _dot(a, b):
    return jnp.dot(a, b, preferred_element_type=F32)


def _phi(t):
    return jnp.where(t > 0, t + 1.0, jnp.exp(t)) + 1e-6


def _radix4(A):
    (r0, i0), (r1, i1), (r2, i2), (r3, i3) = A
    a0r, a0i = r0 + r2, i0 + i2
    a1r, a1i = r0 - r2, i0 - i2
    b0r, b0i = r1 + r3, i1 + i3
    b1r, b1i = r1 - r3, i1 - i3
    return [(a0r + b0r, a0i + b0i), (a1r + b1i, a1i - b1r),
            (a0r - b0r, a0i - b0i), (a1r - b1i, a1i + b1r)]


def _iradix4(W):
    (r0, i0), (r1, i1), (r2, i2), (r3, i3) = W
    c0r, c0i = r0 + r2, i0 + i2
    c1r, c1i = r0 - r2, i0 - i2
    d0r, d0i = r1 + r3, i1 + i3
    d1r, d1i = r1 - r3, i1 - i3
    return [(c0r + d0r, c0i + d0i), (c1r - d1i, c1i + d1r),
            (c0r - d0r, c0i - d0i), (c1r + d1i, c1i - d1r)]


def b_front_x(k_s, v_s, sk, xs, j):
    kw = k_s.bitcast(U32)
    vw = v_s.bitcast(U32)
    s0, s1, s2, s3 = sk
    for n in range(8):
        t0 = 128 * j + 16 * n
        base = 8 + 2 * t0
        E = kw[pl.ds(base, 16, stride=2), :]
        O = kw[pl.ds(base + 1, 16, stride=2), :]
        Ep = kw[pl.ds(base - 2, 16, stride=2), :]
        Op = kw[pl.ds(base - 1, 16, stride=2), :]
        k0, k1, k2, k3 = _lo(E), _hi(E), _lo(O), _hi(O)
        k1p, k2p, k3p = _hi(Ep), _lo(Op), _hi(Op)
        Ev = vw[pl.ds(2 * t0, 16, stride=2), :]
        Ov = vw[pl.ds(2 * t0 + 1, 16, stride=2), :]
        ks0 = s0 * k0 + s1 * k3p + s2 * k2p + s3 * k1p
        ks1 = s0 * k1 + s1 * k0 + s2 * k3p + s3 * k2p
        ks2 = s0 * k2 + s1 * k1 + s2 * k0 + s3 * k3p
        ks3 = s0 * k3 + s1 * k2 + s2 * k1 + s3 * k0
        kv = [ks0 * _lo(Ev), ks1 * _hi(Ev), ks2 * _lo(Ov), ks3 * _hi(Ov)]
        for t2 in range(4):
            xs[t2, j, pl.ds(8 * n, 8), :] = _pk(kv[t2])
        yield 100


def b_front_h(h_s, ht_s, hs, m):
    for tt in range(4):
        c0 = 512 * m + 128 * tt
        ht_s[pl.ds(c0, 128), :] = h_s[:, pl.ds(c0, 128)].T
        yield 40
    hw = ht_s.bitcast(U32)
    m16 = jnp.uint32(0xFFFF)
    mh = jnp.uint32(0xFFFF0000)
    for n in range(8):
        base = 256 * m + 32 * n
        A0 = hw[pl.ds(base + 0, 8, stride=4), :]
        B0 = hw[pl.ds(base + 2, 8, stride=4), :]
        A1 = hw[pl.ds(base + 1, 8, stride=4), :]
        B1 = hw[pl.ds(base + 3, 8, stride=4), :]
        P = [(A0 & m16) | (B0 << 16), (A0 >> 16) | (B0 & mh),
             (A1 & m16) | (B1 << 16), (A1 >> 16) | (B1 & mh)]
        for t2 in range(4):
            hs[t2, m, pl.ds(8 * n, 8), :] = P[t2]
        if n % 4 == 3:
            yield 48


def b_fwd(f_ref, xs, ax, j, dvec=None):
    CH = FWD_CH
    X = [_bf(xs[t2, j]) for t2 in range(4)]

    def finish(ch, A):
        for pp in range(CH // 16):
            p = ch * (CH // 16) + pp
            a = [(A[t2][16 * pp:16 * pp + 8], A[t2][16 * pp + 8:16 * pp + 16]) for t2 in range(4)]
            if dvec is not None:
                a[0] = (a[0][0] + dvec, a[0][1])
            Xk = _radix4(a)
            for k in range(4):
                ax[k, j, pl.ds(16 * p, 8), :] = Xk[k][0]
                ax[k, j, pl.ds(16 * p + 8, 8), :] = Xk[k][1]

    prev = None
    for ch in range(256 // CH):
        A = [_dot(_bf(f_ref[t2, pl.ds(ch * CH // 2, CH // 2), :]), X[t2]) for t2 in range(4)]
        if prev is not None:
            finish(*prev)
        prev = (ch, A)
        yield CH * 5
    finish(*prev)
    yield CH


def b_first(k_s, v_s, h_s, sk, dvec, ht_s, xs, hs, f_ref, ax, ah):
    fx = lambda j: b_front_x(k_s, v_s, sk, xs, j)
    fh = lambda m: b_front_h(h_s, ht_s, hs, m)
    dx = lambda j: b_fwd(f_ref, xs, ax, j)
    dh = lambda m: b_fwd(f_ref, hs, ah, m, dvec if m == 0 else None)
    for g in (fx(0), fx(1), dx(0), fx(2), dx(1), fx(3), dx(2), fh(0), dx(3), fh(1), dh(0), fh(2), dh(1),
              fh(3), dh(2), dh(3)):
        yield from g


BF_TOT = 32 * 100 + 4 * (160 + 96) + 8 * (256 * 5 + FWD_CH)


def b_mid(ax, ah, vs):
    for p in range(16):
        pos = p < 8
        r_re = pl.ds(16 * p, 8)
        r_im = pl.ds(16 * p + 8, 8)
        Zp = None
        for i in range(4):
            Z = []
            for k in range(4):
                wr = None
                wi = None
                for j in range(i + 1):
                    xr, xi = ax[k, j, r_re, :], ax[k, j, r_im, :]
                    gr, gi = ah[k, i - j, r_re, :], ah[k, i - j, r_im, :]
                    pr = xr * gr - xi * gi
                    pi = xr * gi + xi * gr
                    wr = pr if wr is None else wr + pr
                    wi = pi if wi is None else wi + pi
                Z.append((wr, wi))
            if Zp is None:
                W = Z
            elif pos:
                W = [(Z[k][0] - Zp[k][1], Z[k][1] + Zp[k][0]) for k in range(4)]
            else:
                W = [(Z[k][0] + Zp[k][1], Z[k][1] - Zp[k][0]) for k in range(4)]
            Zp = Z
            V = _iradix4(W)
            for t2 in range(4):
                vs[t2, i, pl.ds(8 * p, 8), :] = _pk(jnp.concatenate([V[t2][0], V[t2][1]], axis=0))
            yield 40 + 32 * (i + 1) + (8 if i else 0)


def b_back(vs, finv_ref, q_s, o_s):
    qw = q_s.bitcast(U32)
    ow = o_s.bitcast(U32)
    CH = BACK_CH

    def finish(base, y):
        E = qw[pl.ds(base, CH, stride=2), :]
        ow[pl.ds(base, CH, stride=2), :] = pltpu.pack_elementwise(
            [_lo(E) * y[0], _hi(E) * y[1]], packed_dtype=BF)

    prev = None
    for i in range(4):
        for hf in range(2):
            Vt = [_bf(vs[2 * hf + e, i]) for e in range(2)]
            for ch in range(128 // CH):
                y = [_dot(_bf(finv_ref[2 * hf + e, pl.ds(ch * CH // 2, CH // 2), :]), Vt[e]) for e in range(2)]
                if prev is not None:
                    finish(*prev)
                prev = (256 * i + 2 * CH * ch + hf, y)
                yield CH * 5
    finish(*prev)
    yield CH


def b_second(ax, ah, vs, finv_ref, q_s, o_s):
    yield from b_mid(ax, ah, vs)
    yield from b_back(vs, finv_ref, q_s, o_s)


BS_TOT = 16 * (160 + 320 + 24) + 8 * 128 * 5 + BACK_CH


def a_phase1(x_s, w_s, r0, kv_acc, z_acc):
    def finish(g, kf, vf):
        pk = _phi(kf)
        z_acc[:, pl.ds(128 * g, 128)] += jnp.sum(pk.reshape(MA // 8, 8, 128), axis=0)
        return g, pk.astype(BF), vf.astype(BF)

    def tn(g, pkb, vb):
        kv_acc[g] += lax.dot_general(pkb, vb, (((0,), (0,)), ((), ())), preferred_element_type=F32)

    pend = None
    pend2 = None
    for mc in range(R // MA):
        rw = pl.multiple_of(r0 // 2 + mc * (MA // 2), MA // 2)
        for g in range(8):
            xt = _bf(x_s[pl.ds(rw, MA // 2), :])
            kf = _dot(xt, _bf(w_s[:, pl.ds(1024 + 128 * g, 128)]))
            if pend is not None:
                pend2 = finish(*pend)
                pend = None
            yield 256
            vf = _dot(xt, _bf(w_s[:, pl.ds(2048 + 128 * g, 128)]))
            if pend2 is not None:
                tn(*pend2)
                pend2 = None
            pend = (g, kf, vf)
            yield 256 + 32
    pend2 = finish(*pend)
    yield 16
    tn(*pend2)
    yield 32


A1_TOT = 16 * (512 + 32) + 48


def a_boundary(kv_acc, z_acc, wo_s, m_s, zt_s):
    ri = lax.broadcasted_iota(jnp.int32, (128, 128), 0) // 32
    ci = lax.broadcasted_iota(jnp.int32, (128, 128), 1) // 32
    same = ri == ci
    z = jnp.sum(z_acc[...], axis=0, keepdims=True)
    for g in range(8):
        kvb = jnp.where(same, kv_acc[g], 0.0).astype(BF)
        m_s[pl.ds(64 * g, 64), :] = _pk(_dot(kvb, _bf(wo_s[pl.ds(64 * g, 64), :])))
        zt_s[g] = _pk(jnp.where(same, jnp.broadcast_to(z[:, 128 * g:128 * (g + 1)], (128, 128)), 0.0))


def a_phase2(x_s, w_s, r0, zt_s, m_s, wg_s, oa_s):
    def den_dot(g, mc, qf):
        pq = _phi(qf)
        den = lax.dot_general(pq.astype(BF), _bf(zt_s[g]), (((1,), (1,)), ((), ())),
                              preferred_element_type=F32)
        return g, mc, pq, den

    def fin(g, mc, pq, den):
        wg_s[mc, :, pl.ds(128 * g, 128)] = _pk(pq / (den + 1e-6))

    def out_dot(mc, n):
        wg = _bf(wg_s[mc])
        oa_s[pl.ds(mc * MA, MA), pl.ds(128 * n, 128)] = _dot(wg, _bf(m_s[:, pl.ds(128 * n, 128)])).astype(BF)

    p1 = None
    p2 = None
    nmc = R // MA
    for mc in range(nmc):
        rw = pl.multiple_of(r0 // 2 + mc * (MA // 2), MA // 2)
        for g in range(8):
            xt = _bf(x_s[pl.ds(rw, MA // 2), :])
            qf = _dot(xt, _bf(w_s[:, pl.ds(128 * g, 128)]))
            if p2 is not None:
                fin(*p2)
                p2 = None
            if p1 is not None:
                p2 = den_dot(*p1)
            p1 = (g, mc, qf)
            yield 256 + 32
            if mc > 0 and g >= 2:
                out_dot(mc - 1, g - 2)
                yield 256
        if mc > 0:
            for n in (6, 7):
                out_dot(mc - 1, n)
                yield 256
    fin(*p2)
    p2 = den_dot(*p1)
    yield 32
    fin(*p2)
    yield 16
    for n in range(8):
        out_dot(nmc - 1, n)
        yield 256


A2_TOT = 16 * (256 + 32) + 16 * 256 + 48


def _interleave(a_items, b_items, a_tot, b_tot):
    a_done = 0.0
    b_done = 0.0
    a_alive = True
    b_alive = True
    while a_alive or b_alive:
        fa = a_done / a_tot
        fb = b_done / b_tot
        if b_alive and (not a_alive or fb < fa):
            try:
                b_done += next(b_items)
            except StopIteration:
                b_alive = False
        else:
            try:
                a_done += next(a_items)
            except StopIteration:
                a_alive = False


def _chain(*gens):
    for g in gens:
        yield from g


BM_TOT = 16 * (160 + 320 + 24)
BK_TOT = 8 * 128 * 5 + BACK_CH


def _run(gen):
    for _ in gen:
        pass


def kernel(x_hbm, w_hbm, wo_hbm, q_hbm, k_hbm, v_hbm, h_hbm, skT_ref, d_ref, f_ref, finv_ref, o_hbm,
           x_s, w_s, wo_s, m_s, kv_acc, z_acc, zt_s, wg_s, oa_s,
           q_s, k_s, v_s, h_s, o_s, ht_s, xs, hs, ax, ah, vs, d_s,
           sem_x, sem_w, sem_b, sem_ob, sem_oa):
    def x_cp(i):
        return pltpu.make_async_copy(x_hbm.at[0, pl.ds(i * R, R), :],
                                     x_s.bitcast(BF).at[pl.ds(i * R, R), :], sem_x.at[i])

    def w_cp(i):
        return pltpu.make_async_copy(w_hbm.at[:, pl.ds(i * 1024, 1024)],
                                     w_s.bitcast(BF).at[:, pl.ds(i * 1024, 1024)], sem_w.at[i])

    wo_cp = pltpu.make_async_copy(wo_hbm, wo_s.bitcast(BF), sem_w.at[3])

    def f_in(c):
        col = pl.multiple_of(c * C, C)
        return [
            pltpu.make_async_copy(k_hbm.at[0, :, pl.ds(col, C)], k_s.at[pl.ds(16, S), :], sem_b.at[0]),
            pltpu.make_async_copy(v_hbm.at[0, :, pl.ds(col, C)], v_s.at[pl.ds(0, S), :], sem_b.at[1]),
            pltpu.make_async_copy(h_hbm.at[pl.ds(col, C), :], h_s, sem_b.at[2]),
        ]

    def q_cp(c):
        col = pl.multiple_of(c * C, C)
        return pltpu.make_async_copy(q_hbm.at[0, :, pl.ds(col, C)], q_s.at[pl.ds(0, S), :], sem_b.at[3])

    def ob_cp(c):
        col = pl.multiple_of(D + c * C, C)
        return pltpu.make_async_copy(o_s.at[pl.ds(0, S), :], o_hbm.at[0, :, pl.ds(col, C)], sem_ob.at[0])

    def oa_cp(i, slot):
        r = pl.multiple_of(i * R, R)
        return pltpu.make_async_copy(oa_s.at[slot], o_hbm.at[0, pl.ds(r, R), pl.ds(0, D)], sem_oa.at[slot])

    def gen_f(c):
        col = pl.multiple_of(c * C, C)
        sk = [skT_ref[pl.ds(i, 1), pl.ds(col, C)].astype(F32) for i in range(4)]
        dvec = d_s[:, pl.ds(col, C)]
        return b_first(k_s, v_s, h_s, sk, dvec, ht_s, xs, hs, f_ref, ax, ah)

    def gen_m():
        return b_mid(ax, ah, vs)

    def gen_k():
        return b_back(vs, finv_ref, q_s, o_s)

    def a1(s):
        return a_phase1(x_s, w_s, pl.multiple_of(s * R, R), kv_acc, z_acc)

    def a2(s, slot):
        return a_phase2(x_s, w_s, pl.multiple_of(s * R, R), zt_s, m_s, wg_s, oa_s.at[slot])

    def post_f(c):
        q_cp(c).start()

        @pl.when(c + 1 < NT)
        def _():
            for cp in f_in(c + 1):
                cp.start()

    def pre_kf(c):
        q_cp(c).wait()

        @pl.when(c + 1 < NT)
        def _():
            for cp in f_in(c + 1):
                cp.wait()

        @pl.when(c >= 1)
        def _():
            ob_cp(c - 1).wait()

    for cp in f_in(0):
        cp.start()
    x_cp(0).start()
    w_cp(1).start()
    w_cp(2).start()
    kv_acc[...] = jnp.zeros_like(kv_acc)
    z_acc[...] = jnp.zeros_like(z_acc)
    k_s[pl.ds(0, 16), :] = jnp.zeros((16, C), BF)
    d_s[...] = d_ref[...].reshape(1, D).astype(F32)
    for cp in f_in(0):
        cp.wait()
    _run(gen_f(0))
    w_cp(1).wait()
    w_cp(2).wait()
    x_cp(1).start()
    post_f(0)
    for i in range(2, NR):
        x_cp(i).start()

    def phase1_body(s, carry):
        c = s // 2
        x_cp(s).wait()

        @pl.when(s % 2 == 0)
        def _():
            _interleave(a1(s), gen_m(), A1_TOT, BM_TOT)

        @pl.when(s % 2 == 1)
        def _():
            pre_kf(c)

        @pl.when(s % 2 == 1)
        def _():
            _interleave(a1(s), _chain(gen_k(), gen_f(c + 1)), A1_TOT, BK_TOT + BF_TOT)
            ob_cp(c).start()
            post_f(c + 1)

        @pl.when(s == 1)
        def _():
            w_cp(0).start()
            wo_cp.start()
        return carry

    lax.fori_loop(0, 8, phase1_body, 0)

    w_cp(0).wait()
    wo_cp.wait()
    a_boundary(kv_acc, z_acc, wo_s, m_s, zt_s)

    def phase2_body(s, carry):
        c = 4 + s // 2

        @pl.when(s >= 2)
        def _():
            oa_cp(s - 2, s % 2).wait()

        @pl.when(s % 2 == 0)
        def _():
            _interleave(a2(s, 0), gen_m(), A2_TOT, BM_TOT)
            oa_cp(s, 0).start()

        @pl.when(s % 2 == 1)
        def _():
            pre_kf(c)

        @pl.when(s % 2 == 1)
        def _():
            _interleave(a2(s, 1), _chain(gen_k(), gen_f(c + 1)), A2_TOT, BK_TOT + BF_TOT)
            oa_cp(s, 1).start()
            ob_cp(c).start()
            post_f(c + 1)
        return carry

    lax.fori_loop(0, 7, phase2_body, 0)
    oa_cp(5, 1).wait()
    pre_kf(7)
    _interleave(a2(7, 1), gen_k(), A2_TOT, BK_TOT)
    oa_cp(7, 1).start()
    ob_cp(7).start()
    oa_cp(6, 0).wait()
    oa_cp(7, 1).wait()
    ob_cp(7).wait()


@jax.jit
def pallas_concat_heads__linear_attn_block__ssm_conv_h3__prompt_kernel(A_x, A_wqkv, A_wo, B_q, B_k, B_v, B_shift_k, B_ssm_k, B_ssm_D):
    any_spec = pl.BlockSpec(memory_space=pl.ANY)
    vm = pl.BlockSpec(memory_space=pltpu.VMEM)
    return pl.pallas_call(
        kernel,
        in_specs=[any_spec] * 7 + [vm, vm, vm, vm],
        out_specs=any_spec,
        out_shape=jax.ShapeDtypeStruct((1, S, 2 * D), BF),
        scratch_shapes=[
            pltpu.VMEM((S // 2, D), U32),
            pltpu.VMEM((D // 2, 3 * D), U32),
            pltpu.VMEM((D // 2, D), U32),
            pltpu.VMEM((D // 2, D), U32),
            pltpu.VMEM((8, 128, 128), F32),
            pltpu.VMEM((8, D), F32),
            pltpu.VMEM((8, 64, 128), U32),
            pltpu.VMEM((R // MA, MA // 2, D), U32),
            pltpu.VMEM((2, R, D), BF),
            pltpu.VMEM((S + 16, C), BF),
            pltpu.VMEM((S + 32, C), BF),
            pltpu.VMEM((S + 16, C), BF),
            pltpu.VMEM((C, S), BF),
            pltpu.VMEM((S + 16, C), BF),
            pltpu.VMEM((S + 16, C), BF),
            pltpu.VMEM((4, 4, 64, 128), U32),
            pltpu.VMEM((4, 4, 64, 128), U32),
            pltpu.VMEM((4, 4, 256, 128), F32),
            pltpu.VMEM((4, 4, 256, 128), F32),
            pltpu.VMEM((4, 4, 128, 128), U32),
            pltpu.VMEM((1, D), F32),
            pltpu.SemaphoreType.DMA((NR,)),
            pltpu.SemaphoreType.DMA((4,)),
            pltpu.SemaphoreType.DMA((4,)),
            pltpu.SemaphoreType.DMA((1,)),
            pltpu.SemaphoreType.DMA((2,)),
        ],
        compiler_params=pltpu.CompilerParams(vmem_limit_bytes=100 * 1024 * 1024),
        name="fused",
    )(A_x, A_wqkv, A_wo, B_q, B_k, B_v, B_ssm_k, B_shift_k.T, B_ssm_D,
      jnp.asarray(_F_PK), jnp.asarray(_FINV_PK))
```

```python
import numpy as np
import jax
import jax.numpy as jnp
from jax import lax
from jax.experimental import pallas as pl
from jax.experimental.pallas import tpu as pltpu

S, D = 2048, 1024
C = 128
NT = D // C
MF = 1024
R = 256
NR = S // R
MA = 128
BF = jnp.bfloat16
F32 = jnp.float32
U32 = jnp.uint32

FWD_CH = 128
BACK_CH = 64


def _make_consts():
    p = np.arange(16)[:, None]
    s = np.arange(8)[None, :]
    k1 = np.where(p < 8, 2 * (8 * p + s), 2 * (8 * (p - 8) + s) + 1)
    t1 = np.arange(128)
    F = np.zeros((4, 256, 128), np.float64)
    for t2 in range(4):
        th = 2 * np.pi * (4 * t1[None, None, :] + t2) * (k1[:, :, None] + 0.5) / MF
        F[t2] = np.stack([np.cos(th), -np.sin(th)], axis=1).reshape(256, 128)
    Finv = np.transpose(F, (0, 2, 1)) * (2.0 / MF)
    return F.astype(np.float32), Finv.astype(np.float32)


def _pack_rows(a):
    a = np.ascontiguousarray(a, np.float32)
    u = a.view(np.uint32)
    b = ((u + 0x7FFF + ((u >> 16) & 1)) >> 16).astype(np.uint32)
    return (b[..., 0::2, :] | (b[..., 1::2, :] << 16)).astype(np.uint32)


_F_NP, _FINV_NP = _make_consts()
_F_PK = _pack_rows(_F_NP)
_FINV_PK = _pack_rows(_FINV_NP)


def _lo(w):
    return pltpu.bitcast(w << 16, F32)


def _hi(w):
    return pltpu.bitcast(w & jnp.uint32(0xFFFF0000), F32)


def _bf(w):
    return pltpu.bitcast(w, BF)


def _pk(v):
    return pltpu.bitcast(v.astype(BF), U32)


def _dot(a, b):
    return jnp.dot(a, b, preferred_element_type=F32)


def _phi(t):
    return jnp.where(t > 0, t + 1.0, jnp.exp(t)) + 1e-6


def _radix4(A):
    (r0, i0), (r1, i1), (r2, i2), (r3, i3) = A
    a0r, a0i = r0 + r2, i0 + i2
    a1r, a1i = r0 - r2, i0 - i2
    b0r, b0i = r1 + r3, i1 + i3
    b1r, b1i = r1 - r3, i1 - i3
    return [(a0r + b0r, a0i + b0i), (a1r + b1i, a1i - b1r),
            (a0r - b0r, a0i - b0i), (a1r - b1i, a1i + b1r)]


def _iradix4(W):
    (r0, i0), (r1, i1), (r2, i2), (r3, i3) = W
    c0r, c0i = r0 + r2, i0 + i2
    c1r, c1i = r0 - r2, i0 - i2
    d0r, d0i = r1 + r3, i1 + i3
    d1r, d1i = r1 - r3, i1 - i3
    return [(c0r + d0r, c0i + d0i), (c1r - d1i, c1i + d1r),
            (c0r - d0r, c0i - d0i), (c1r + d1i, c1i - d1r)]


def b_front_x(k_s, v_s, sk, xs, j):
    kw = k_s.bitcast(U32)
    vw = v_s.bitcast(U32)
    s0, s1, s2, s3 = sk
    for n in range(8):
        t0 = 128 * j + 16 * n
        base = 8 + 2 * t0
        E = kw[pl.ds(base, 16, stride=2), :]
        O = kw[pl.ds(base + 1, 16, stride=2), :]
        Ep = kw[pl.ds(base - 2, 16, stride=2), :]
        Op = kw[pl.ds(base - 1, 16, stride=2), :]
        k0, k1, k2, k3 = _lo(E), _hi(E), _lo(O), _hi(O)
        k1p, k2p, k3p = _hi(Ep), _lo(Op), _hi(Op)
        Ev = vw[pl.ds(2 * t0, 16, stride=2), :]
        Ov = vw[pl.ds(2 * t0 + 1, 16, stride=2), :]
        ks0 = s0 * k0 + s1 * k3p + s2 * k2p + s3 * k1p
        ks1 = s0 * k1 + s1 * k0 + s2 * k3p + s3 * k2p
        ks2 = s0 * k2 + s1 * k1 + s2 * k0 + s3 * k3p
        ks3 = s0 * k3 + s1 * k2 + s2 * k1 + s3 * k0
        kv = [ks0 * _lo(Ev), ks1 * _hi(Ev), ks2 * _lo(Ov), ks3 * _hi(Ov)]
        for t2 in range(4):
            xs[t2, j, pl.ds(8 * n, 8), :] = _pk(kv[t2])
        yield 100


def b_front_h(h_s, ht_s, hs, m):
    for tt in range(4):
        c0 = 512 * m + 128 * tt
        ht_s[pl.ds(c0 // 2, 64), :] = pltpu.bitcast(_bf(h_s[:, pl.ds(c0, 128)]).T, U32)
        yield 40
    hw = ht_s
    m16 = jnp.uint32(0xFFFF)
    mh = jnp.uint32(0xFFFF0000)
    for n in range(8):
        base = 256 * m + 32 * n
        A0 = hw[pl.ds(base + 0, 8, stride=4), :]
        B0 = hw[pl.ds(base + 2, 8, stride=4), :]
        A1 = hw[pl.ds(base + 1, 8, stride=4), :]
        B1 = hw[pl.ds(base + 3, 8, stride=4), :]
        P = [(A0 & m16) | (B0 << 16), (A0 >> 16) | (B0 & mh),
             (A1 & m16) | (B1 << 16), (A1 >> 16) | (B1 & mh)]
        for t2 in range(4):
            hs[t2, m, pl.ds(8 * n, 8), :] = P[t2]
        if n % 4 == 3:
            yield 48


def b_fwd(f_ref, xs, ax, j, dvec=None):
    CH = FWD_CH
    X = [_bf(xs[t2, j]) for t2 in range(4)]

    def finish(ch, A):
        for pp in range(CH // 16):
            p = ch * (CH // 16) + pp
            a = [(A[t2][16 * pp:16 * pp + 8], A[t2][16 * pp + 8:16 * pp + 16]) for t2 in range(4)]
            if dvec is not None:
                a[0] = (a[0][0] + dvec, a[0][1])
            Xk = _radix4(a)
            for k in range(4):
                ax[k, j, pl.ds(16 * p, 8), :] = Xk[k][0]
                ax[k, j, pl.ds(16 * p + 8, 8), :] = Xk[k][1]

    prev = None
    for ch in range(256 // CH):
        A = [_dot(_bf(f_ref[t2, pl.ds(ch * CH // 2, CH // 2), :]), X[t2]) for t2 in range(4)]
        if prev is not None:
            finish(*prev)
        prev = (ch, A)
        yield CH * 5
    finish(*prev)
    yield CH


def _call(fn):
    if fn is not None:
        fn()
    yield 0


def b_first(k_s, v_s, h_s, sk, dvec, ht_s, xs, hs, f_ref, ax, ah, wait_x=None, wait_h=None):
    fx = lambda j: b_front_x(k_s, v_s, sk, xs, j)
    fh = lambda m: b_front_h(h_s, ht_s, hs, m)
    dx = lambda j: b_fwd(f_ref, xs, ax, j)
    dh = lambda m: b_fwd(f_ref, hs, ah, m, dvec if m == 0 else None)
    for g in (_call(wait_x), fx(0), fx(1), dx(0), fx(2), dx(1), fx(3), dx(2), _call(wait_h), fh(0), dx(3), fh(1),
              dh(0), fh(2), dh(1), fh(3), dh(2), dh(3)):
        yield from g


BF_TOT = 32 * 100 + 4 * (160 + 96) + 8 * (256 * 5 + FWD_CH)


def b_mid(ax, ah, vs):
    for p in range(16):
        pos = p < 8
        r_re = pl.ds(16 * p, 8)
        r_im = pl.ds(16 * p + 8, 8)
        Zp = None
        for i in range(4):
            Z = []
            for k in range(4):
                wr = None
                wi = None
                for j in range(i + 1):
                    xr, xi = ax[k, j, r_re, :], ax[k, j, r_im, :]
                    gr, gi = ah[k, i - j, r_re, :], ah[k, i - j, r_im, :]
                    pr = xr * gr - xi * gi
                    pi = xr * gi + xi * gr
                    wr = pr if wr is None else wr + pr
                    wi = pi if wi is None else wi + pi
                Z.append((wr, wi))
            if Zp is None:
                W = Z
            elif pos:
                W = [(Z[k][0] - Zp[k][1], Z[k][1] + Zp[k][0]) for k in range(4)]
            else:
                W = [(Z[k][0] + Zp[k][1], Z[k][1] - Zp[k][0]) for k in range(4)]
            Zp = Z
            V = _iradix4(W)
            for t2 in range(4):
                vs[t2, i, pl.ds(8 * p, 8), :] = _pk(jnp.concatenate([V[t2][0], V[t2][1]], axis=0))
            yield 40 + 32 * (i + 1) + (8 if i else 0)


def b_back(vs, finv_ref, q_s, o_s, blocks=range(4)):
    qw = q_s.bitcast(U32)
    ow = o_s.bitcast(U32)
    CH = BACK_CH

    def finish(base, y):
        E = qw[pl.ds(base, CH, stride=2), :]
        ow[pl.ds(base, CH, stride=2), :] = pltpu.pack_elementwise(
            [_lo(E) * y[0], _hi(E) * y[1]], packed_dtype=BF)

    prev = None
    for i in blocks:
        for hf in range(2):
            Vt = [_bf(vs[2 * hf + e, i]) for e in range(2)]
            for ch in range(128 // CH):
                y = [_dot(_bf(finv_ref[2 * hf + e, pl.ds(ch * CH // 2, CH // 2), :]), Vt[e]) for e in range(2)]
                if prev is not None:
                    finish(*prev)
                prev = (256 * i + 2 * CH * ch + hf, y)
                yield CH * 5
    finish(*prev)
    yield CH


def _tn(kv_acc, g, pkb, vb):
    kv_acc[g] += lax.dot_general(pkb, vb, (((0,), (0,)), ((), ())), preferred_element_type=F32)


def _tn_deferred(kv_acc, g, pb_s):
    _tn(kv_acc, g, _bf(pb_s[0]), _bf(pb_s[1]))


def _kv_finish(z_acc, col, kf, vf):
    pk = _phi(kf)
    z_acc[:, pl.ds(col, 128)] += jnp.sum(pk.reshape(MA // 8, 8, 128), axis=0)
    return pk.astype(BF), vf.astype(BF)


def a_phase1(x_s, w_s, r0, kv_acc, z_acc, pb_s):
    pend = None
    pend2 = None
    for mc in range(R // MA):
        rw = pl.multiple_of(r0 // 2 + mc * (MA // 2), MA // 2)
        for g in range(8):
            xt = _bf(x_s[pl.ds(rw, MA // 2), :])
            kf = _dot(xt, _bf(w_s[:, pl.ds(1024 + 128 * g, 128)]))
            if mc == 0 and g == 0:
                _tn_deferred(kv_acc, 7, pb_s)
            if pend is not None:
                pend2 = (pend[0],) + _kv_finish(z_acc, 128 * pend[0], pend[1], pend[2])
                pend = None
            yield 256
            vf = _dot(xt, _bf(w_s[:, pl.ds(2048 + 128 * g, 128)]))
            if pend2 is not None:
                _tn(kv_acc, *pend2)
                pend2 = None
            pend = (g, kf, vf)
            yield 256 + 32
    pkb, vb = _kv_finish(z_acc, 128 * pend[0], pend[1], pend[2])
    pb_s[0] = pltpu.bitcast(pkb, U32)
    pb_s[1] = pltpu.bitcast(vb, U32)
    yield 16


A1_TOT = 16 * (512 + 32) + 16


def a_boundary_prep(kv_acc, z_acc, kvb_s, zt_s):
    ri = lax.broadcasted_iota(jnp.int32, (128, 128), 0) // 32
    ci = lax.broadcasted_iota(jnp.int32, (128, 128), 1) // 32
    same = ri == ci
    z = jnp.sum(z_acc[...], axis=0, keepdims=True)
    for g in range(8):
        kvb_s[g] = _pk(jnp.where(same, kv_acc[g], 0.0))
        zt_s[g] = _pk(jnp.where(same, jnp.broadcast_to(z[:, 128 * g:128 * (g + 1)], (128, 128)), 0.0))


def a_boundary(kvb_s, wo_s, m_s):
    for g in range(8):
        for hf in range(4):
            cs = pl.ds(256 * hf, 256)
            m_s[pl.ds(64 * g, 64), cs] = _pk(_dot(_bf(kvb_s[g]), _bf(wo_s[pl.ds(64 * g, 64), cs])))
            yield 64


def a_phase2(x_s, w_s, r0, zt_s, m_s, wg_s, oa_s):
    def den_dot(g, mc, qf):
        pq = _phi(qf)
        den = lax.dot_general(pq.astype(BF), _bf(zt_s[g]), (((1,), (1,)), ((), ())),
                              preferred_element_type=F32)
        return g, mc, pq, den

    def fin(g, mc, pq, den):
        wg_s[mc, :, pl.ds(128 * g, 128)] = _pk(pq * pl.reciprocal(den + 1e-6, approx=True))

    def out_dot(mc, n):
        wg = _bf(wg_s[mc])
        oa_s[pl.ds(mc * (MA // 2), MA // 2), pl.ds(128 * n, 128)] = _pk(_dot(wg, _bf(m_s[:, pl.ds(128 * n, 128)])))

    p1 = None
    p2 = None
    nmc = R // MA
    for mc in range(nmc):
        rw = pl.multiple_of(r0 // 2 + mc * (MA // 2), MA // 2)
        for g in range(8):
            xt = _bf(x_s[pl.ds(rw, MA // 2), :])
            qf = _dot(xt, _bf(w_s[:, pl.ds(128 * g, 128)]))
            if p2 is not None:
                fin(*p2)
                p2 = None
            if p1 is not None:
                p2 = den_dot(*p1)
            p1 = (g, mc, qf)
            yield 256 + 32
            if mc > 0 and g >= 3:
                out_dot(mc - 1, g - 3)
                yield 256
    out_dot(nmc - 2, 5)
    fin(*p2)
    yield 256
    p2 = den_dot(*p1)
    out_dot(nmc - 2, 6)
    yield 256 + 32
    out_dot(nmc - 2, 7)
    fin(*p2)
    yield 256
    for n in range(8):
        out_dot(nmc - 1, n)
        yield 256


A2_TOT = 16 * (256 + 32) + 16 * 256


def _interleave(a_items, b_items, a_tot, b_tot, lead=0.0, tail=0.0):
    a_done = 0.0
    b_done = 0.0
    a_alive = True
    b_alive = True
    while a_alive or b_alive:
        fa = (a_done / a_tot - lead) / (1.0 - lead - tail)
        fb = b_done / b_tot
        if b_alive and (not a_alive or fb < fa):
            try:
                b_done += next(b_items)
            except StopIteration:
                b_alive = False
        else:
            try:
                a_done += next(a_items)
            except StopIteration:
                a_alive = False


def _chain(*gens):
    for g in gens:
        yield from g


BM_TOT = 16 * (160 + 320 + 24)
BK_TOT = 8 * 128 * 5 + BACK_CH
STAGE2_AT = 5
A1F_LEAD = 0.2
BD_TOT = 8 * 256


def _run(gen):
    for _ in gen:
        pass


def a_start(x_s, w_s, kv_acc, z_acc, pb_s, wait_chunk):
    pb_s[...] = jnp.zeros_like(pb_s)

    def body(g, carry):
        wait_chunk(g)
        ck = pl.multiple_of(1024 + 128 * g, 128)
        cv = pl.multiple_of(2048 + 128 * g, 128)
        col = pl.multiple_of(128 * g, 128)
        x0 = _bf(x_s[pl.ds(0, MA // 2), :])
        x1 = _bf(x_s[pl.ds(MA // 2, MA // 2), :])
        kf0 = _dot(x0, _bf(w_s[:, pl.ds(ck, 128)]))
        _tn_deferred(kv_acc, jnp.maximum(g - 1, 0), pb_s)
        kf1 = _dot(x1, _bf(w_s[:, pl.ds(ck, 128)]))
        vf0 = _dot(x0, _bf(w_s[:, pl.ds(cv, 128)]))
        vf1 = _dot(x1, _bf(w_s[:, pl.ds(cv, 128)]))
        _tn(kv_acc, g, *_kv_finish(z_acc, col, kf0, vf0))
        pkb, vb = _kv_finish(z_acc, col, kf1, vf1)
        pb_s[0] = pltpu.bitcast(pkb, U32)
        pb_s[1] = pltpu.bitcast(vb, U32)
        return carry

    lax.fori_loop(0, 8, body, 0)


def kernel(x_hbm, w_hbm, wo_hbm, q_hbm, k_hbm, v_hbm, h_hbm, skT_hbm, d_hbm, f_hbm, finv_hbm, o_hbm,
           x_s, w_s, wo_s, m_s, kv_acc, z_acc, zt_s, wg_s, oa_s,
           q_s, k_s, v_s, h_s, o_s, ht_s, xs, hs, ax, ah, vs, d_s,
           skT_ref, d_ref, f_ref, finv_ref, pb_s, kvb_s, flag_s,
           sem_x, sem_w, sem_wc, sem_c, sem_b, sem_ob, sem_oa):
    def x_cp(i):
        return pltpu.make_async_copy(x_hbm.at[0, pl.ds(i * R, R), :],
                                     x_s.bitcast(BF).at[pl.ds(i * R, R), :], sem_x.at[i])

    def wc_cp(g, e):
        col = pl.multiple_of(1024 * (1 + e) + 128 * g, 128)
        return pltpu.make_async_copy(w_hbm.at[:, pl.ds(col, 128)],
                                     w_s.bitcast(BF).at[:, pl.ds(col, 128)], sem_wc.at[2 * g + e])

    wq_cp = pltpu.make_async_copy(w_hbm.at[:, pl.ds(0, 1024)], w_s.bitcast(BF).at[:, pl.ds(0, 1024)], sem_w.at[0])
    wo_cp = pltpu.make_async_copy(wo_hbm, wo_s.bitcast(BF), sem_w.at[1])
    c_cps = [pltpu.make_async_copy(skT_hbm, skT_ref, sem_c.at[0]),
             pltpu.make_async_copy(d_hbm, d_ref, sem_c.at[1]),
             pltpu.make_async_copy(f_hbm, f_ref, sem_c.at[2]),
             pltpu.make_async_copy(finv_hbm, finv_ref, sem_c.at[3])]

    def f_in(c):
        col = pl.multiple_of(c * C, C)
        return [
            pltpu.make_async_copy(k_hbm.at[0, :, pl.ds(col, C)], k_s.at[c % 2, pl.ds(16, S), :], sem_b.at[4 * (c % 2) + 0]),
            pltpu.make_async_copy(v_hbm.at[0, :, pl.ds(col, C)], v_s.at[c % 2, pl.ds(0, S), :], sem_b.at[4 * (c % 2) + 1]),
            pltpu.make_async_copy(h_hbm.at[pl.ds(col, C), :], h_s.bitcast(BF).at[c % 2], sem_b.at[4 * (c % 2) + 2]),
        ]

    def q_cp(c):
        col = pl.multiple_of(c * C, C)
        return pltpu.make_async_copy(q_hbm.at[0, :, pl.ds(col, C)], q_s.at[c % 2, pl.ds(0, S), :],
                                     sem_b.at[4 * (c % 2) + 3])

    def ob_cp(c):
        col = pl.multiple_of(D + c * C, C)
        return pltpu.make_async_copy(o_s.at[pl.ds(0, S), :], o_hbm.at[0, :, pl.ds(col, C)], sem_ob.at[0])

    def ob_last_cp(i):
        return pltpu.make_async_copy(o_s.at[pl.ds(512 * i, 512), :],
                                     o_hbm.at[0, pl.ds(512 * i, 512), pl.ds(D + (NT - 1) * C, C)], sem_ob.at[1 + i])

    def oa_cp(i, slot):
        r = pl.multiple_of(i * R, R)
        return pltpu.make_async_copy(oa_s.bitcast(BF).at[slot], o_hbm.at[0, pl.ds(r, R), pl.ds(0, D)], sem_oa.at[slot])

    def gen_f(c, wait_x=None, wait_h=None):
        col = pl.multiple_of(c * C, C)
        sk = [skT_ref[pl.ds(i, 1), pl.ds(col, C)].astype(F32) for i in range(4)]
        dvec = d_s[:, pl.ds(col, C)]
        sl = c % 2
        return b_first(k_s.at[sl], v_s.at[sl], h_s.at[sl], sk, dvec, ht_s, xs, hs, f_ref, ax, ah, wait_x, wait_h)

    def gen_m():
        return b_mid(ax, ah, vs)

    def gen_k(c, blocks=range(4)):
        return b_back(vs, finv_ref, q_s.at[c % 2], o_s, blocks)

    def a1(s):
        return a_phase1(x_s, w_s, pl.multiple_of(s * R, R), kv_acc, z_acc, pb_s)

    def a2(s, slot):
        return a_phase2(x_s, w_s, pl.multiple_of(s * R, R), zt_s, m_s, wg_s, oa_s.at[slot])

    def post_f(c):
        @pl.when(c + 1 < NT)
        def _():
            q_cp(c + 1).start()

        @pl.when(c + 2 < NT)
        def _():
            for cp in f_in(c + 2):
                cp.start()

    def pre_kf(c):
        q_cp(c).wait()

        @pl.when(c + 1 < NT)
        def _():
            for cp in f_in(c + 1):
                cp.wait()

        @pl.when(c >= 1)
        def _():
            ob_cp(c - 1).wait()

    flag_s[0] = 1
    x_cp(0).start()
    for g in range(8):
        wc_cp(g, 0).start()
        wc_cp(g, 1).start()
    kv_acc[...] = jnp.zeros_like(kv_acc)
    z_acc[...] = jnp.zeros_like(z_acc)
    for sl in range(2):
        k_s[sl, pl.ds(0, 16), :] = jnp.zeros((16, C), BF)
    with jax.named_scope("w_x0"):
        x_cp(0).wait()

    def wait_chunk(g):
        wc_cp(g, 0).wait()
        wc_cp(g, 1).wait()

        @pl.when(g == STAGE2_AT)
        def _():
            x_cp(1).start()
            for cp in c_cps:
                cp.start()
            for cp in f_in(0):
                cp.start()

    with jax.named_scope("s0"):
        a_start(x_s, w_s, kv_acc, z_acc, pb_s, wait_chunk)
    x_cp(2).start()
    q_cp(0).start()
    for cp in f_in(1):
        cp.start()
    with jax.named_scope("w_c"):
        x_cp(1).wait()
        for cp in c_cps[:3]:
            cp.wait()
    d_s[...] = d_ref[...].reshape(1, D).astype(F32)

    def wait_kv0():
        for cp in f_in(0)[:2]:
            cp.wait()

    def wait_h0():
        f_in(0)[2].wait()

    with jax.named_scope("a1f"):
        _interleave(a1(1), gen_f(0, wait_kv0, wait_h0), A1_TOT, BF_TOT, lead=A1F_LEAD)
    post_f(0)
    for i in range(3, NR):
        x_cp(i).start()
    wq_cp.start()
    wo_cp.start()
    c_cps[3].wait()

    def phase1_body(s, carry):
        c = (s - 2) // 2
        x_cp(s).wait()

        @pl.when(s % 2 == 0)
        def _():
            with jax.named_scope("a1m"):
                _interleave(a1(s), gen_m(), A1_TOT, BM_TOT)

        @pl.when(s % 2 == 1)
        def _():
            pre_kf(c)

        @pl.when(s % 2 == 1)
        def _():
            with jax.named_scope("a1kf"):
                _interleave(a1(s), _chain(gen_k(c), gen_f(c + 1)), A1_TOT, BK_TOT + BF_TOT)

        @pl.when(flag_s[0] + s % 2 == 2)
        def _():
            ob_cp(c).start()
            post_f(c + 1)
        return carry

    lax.fori_loop(2, 8, phase1_body, 0)

    wq_cp.wait()
    wo_cp.wait()
    with jax.named_scope("bdprep"):
        _tn_deferred(kv_acc, 7, pb_s)
        a_boundary_prep(kv_acc, z_acc, kvb_s, zt_s)

    @pl.when(flag_s[0] == 1)
    def _():
        with jax.named_scope("bd"):
            _interleave(a_boundary(kvb_s, wo_s, m_s), gen_m(), BD_TOT, BM_TOT)


    def phase2_body(s, carry):
        c = 3 + s // 2

        @pl.when(s >= 2)
        def _():
            oa_cp(s - 2, s % 2).wait()

        @pl.when(s % 2 == 0)
        def _():
            pre_kf(c)

        @pl.when(s % 2 == 0)
        def _():
            with jax.named_scope("a2kf"):
                _interleave(a2(s, 0), _chain(gen_k(c), gen_f(c + 1)), A2_TOT, BK_TOT + BF_TOT)

        @pl.when(s % 2 == 1)
        def _():
            with jax.named_scope("a2m"):
                _interleave(a2(s, 1), gen_m(), A2_TOT, BM_TOT)

        @pl.when(flag_s[0] + s % 2 == 1)
        def _():
            oa_cp(s, 0).start()
            ob_cp(c).start()
            post_f(c + 1)

        @pl.when(flag_s[0] + s % 2 == 2)
        def _():
            oa_cp(s, 1).start()
        return carry

    lax.fori_loop(0, 8, phase2_body, 0)
    q_cp(7).wait()
    ob_cp(6).wait()

    with jax.named_scope("lastk"):
        for i in range(4):
            _run(gen_k(NT - 1, [i]))
            ob_last_cp(i).start()
    with jax.named_scope("endwait"):
        oa_cp(6, 0).wait()
        oa_cp(7, 1).wait()
        for i in range(4):
            ob_last_cp(i).wait()


@jax.jit
def pallas_concat_heads__linear_attn_block__ssm_conv_h3__prompt_kernel(A_x, A_wqkv, A_wo, B_q, B_k, B_v, B_shift_k, B_ssm_k, B_ssm_D):
    any_spec = pl.BlockSpec(memory_space=pl.ANY)
    return pl.pallas_call(
        kernel,
        in_specs=[any_spec] * 11,
        out_specs=any_spec,
        out_shape=jax.ShapeDtypeStruct((1, S, 2 * D), BF),
        scratch_shapes=[
            pltpu.VMEM((S // 2, D), U32),
            pltpu.VMEM((D // 2, 3 * D), U32),
            pltpu.VMEM((D // 2, D), U32),
            pltpu.VMEM((D // 2, D), U32),
            pltpu.VMEM((8, 128, 128), F32),
            pltpu.VMEM((8, D), F32),
            pltpu.VMEM((8, 64, 128), U32),
            pltpu.VMEM((R // MA, MA // 2, D), U32),
            pltpu.VMEM((2, R // 2, D), U32),
            pltpu.VMEM((2, S + 16, C), BF),
            pltpu.VMEM((2, S + 32, C), BF),
            pltpu.VMEM((2, S + 16, C), BF),
            pltpu.VMEM((2, C // 2, S), U32),
            pltpu.VMEM((S + 16, C), BF),
            pltpu.VMEM((S // 2 + 8, C), U32),
            pltpu.VMEM((4, 4, 64, 128), U32),
            pltpu.VMEM((4, 4, 64, 128), U32),
            pltpu.VMEM((4, 4, 256, 128), F32),
            pltpu.VMEM((4, 4, 256, 128), F32),
            pltpu.VMEM((4, 4, 128, 128), U32),
            pltpu.VMEM((1, D), F32),
            pltpu.VMEM((4, D), BF),
            pltpu.VMEM((D,), BF),
            pltpu.VMEM((4, 128, 128), U32),
            pltpu.VMEM((4, 64, 256), U32),
            pltpu.VMEM((2, MA // 2, 128), U32),
            pltpu.VMEM((8, 64, 128), U32),
            pltpu.SMEM((1,), jnp.int32),
            pltpu.SemaphoreType.DMA((NR,)),
            pltpu.SemaphoreType.DMA((2,)),
            pltpu.SemaphoreType.DMA((16,)),
            pltpu.SemaphoreType.DMA((4,)),
            pltpu.SemaphoreType.DMA((8,)),
            pltpu.SemaphoreType.DMA((5,)),
            pltpu.SemaphoreType.DMA((2,)),
        ],
        compiler_params=pltpu.CompilerParams(vmem_limit_bytes=100 * 1024 * 1024, disable_bounds_checks=True, disable_semaphore_checks=True),
        name="fused",
    )(A_x, A_wqkv, A_wo, B_q, B_k, B_v, B_ssm_k, B_shift_k.T, B_ssm_D,
      jnp.asarray(_F_PK), jnp.asarray(_FINV_PK))
```

```python
import numpy as np
import jax
import jax.numpy as jnp
from jax import lax
from jax.experimental import pallas as pl
from jax.experimental.pallas import tpu as pltpu

S, D = 2048, 1024
C = 128
NT = D // C
MF = 1024
R = 256
NR = S // R
MA = 128
BF = jnp.bfloat16
F32 = jnp.float32
U32 = jnp.uint32

A2_WQ = 256
A2_WO = 256
NORM_GROUP = 16
FWD_CH = 128
BACK_CH = 64


def _make_consts():
    p = np.arange(16)[:, None]
    s = np.arange(8)[None, :]
    k1 = np.where(p < 8, 2 * (8 * p + s), 2 * (8 * (p - 8) + s) + 1)
    t1 = np.arange(128)
    F = np.zeros((4, 256, 128), np.float64)
    for t2 in range(4):
        th = 2 * np.pi * (4 * t1[None, None, :] + t2) * (k1[:, :, None] + 0.5) / MF
        F[t2] = np.stack([np.cos(th), -np.sin(th)], axis=1).reshape(256, 128)
    Finv = np.transpose(F.reshape(4, 16, 2, 8, 128), (0, 4, 1, 3, 2)).reshape(4, 128, 256) * (2.0 / MF)
    c = np.arange(128)
    perm = 16 * (c // 16) + 8 * (c % 2) + (c % 16) // 2
    F = F[:, :, perm]
    return F.astype(np.float32), Finv.astype(np.float32)


def _pack_rows(a):
    a = np.ascontiguousarray(a, np.float32)
    u = a.view(np.uint32)
    b = ((u + 0x7FFF + ((u >> 16) & 1)) >> 16).astype(np.uint32)
    return (b[..., 0::2, :] | (b[..., 1::2, :] << 16)).astype(np.uint32)


_F_NP, _FINV_NP = _make_consts()
_F_PK = _pack_rows(_F_NP)
_FINV_PK = _pack_rows(_FINV_NP)


def _lo(w):
    return pltpu.bitcast(w << 16, F32)


def _hi(w):
    return pltpu.bitcast(w & jnp.uint32(0xFFFF0000), F32)


def _bf(w):
    return pltpu.bitcast(w, BF)


def _pk(v):
    return pltpu.bitcast(v.astype(BF), U32)


def _dot(a, b):
    return jnp.dot(a, b, preferred_element_type=F32)


def _phi(t):
    return jnp.where(t > 0, t + 1.0, jnp.exp(t)) + 1e-6


def _radix4(A):
    (r0, i0), (r1, i1), (r2, i2), (r3, i3) = A
    a0r, a0i = r0 + r2, i0 + i2
    a1r, a1i = r0 - r2, i0 - i2
    b0r, b0i = r1 + r3, i1 + i3
    b1r, b1i = r1 - r3, i1 - i3
    return [(a0r + b0r, a0i + b0i), (a1r + b1i, a1i - b1r),
            (a0r - b0r, a0i - b0i), (a1r - b1i, a1i + b1r)]


def _iradix4(W):
    (r0, i0), (r1, i1), (r2, i2), (r3, i3) = W
    c0r, c0i = r0 + r2, i0 + i2
    c1r, c1i = r0 - r2, i0 - i2
    d0r, d0i = r1 + r3, i1 + i3
    d1r, d1i = r1 - r3, i1 - i3
    return [(c0r + d0r, c0i + d0i), (c1r - d1i, c1i + d1r),
            (c0r - d0r, c0i - d0i), (c1r + d1i, c1i - d1r)]


def b_front_x(k_s, v_s, sk, xs, j):
    kw = k_s.bitcast(U32)
    vw = v_s.bitcast(U32)
    s0, s1, s2, s3 = sk
    for n in range(8):
        t0 = 128 * j + 16 * n
        base = 8 + 2 * t0
        E = kw[pl.ds(base, 16, stride=2), :]
        O = kw[pl.ds(base + 1, 16, stride=2), :]
        Ep = kw[pl.ds(base - 2, 16, stride=2), :]
        Op = kw[pl.ds(base - 1, 16, stride=2), :]
        k0, k1, k2, k3 = _lo(E), _hi(E), _lo(O), _hi(O)
        k1p, k2p, k3p = _hi(Ep), _lo(Op), _hi(Op)
        Ev = vw[pl.ds(2 * t0, 16, stride=2), :]
        Ov = vw[pl.ds(2 * t0 + 1, 16, stride=2), :]
        ks0 = s0 * k0 + s1 * k3p + s2 * k2p + s3 * k1p
        ks1 = s0 * k1 + s1 * k0 + s2 * k3p + s3 * k2p
        ks2 = s0 * k2 + s1 * k1 + s2 * k0 + s3 * k3p
        ks3 = s0 * k3 + s1 * k2 + s2 * k1 + s3 * k0
        kv = [ks0 * _lo(Ev), ks1 * _hi(Ev), ks2 * _lo(Ov), ks3 * _hi(Ov)]
        for t2 in range(4):
            xs[t2, j, pl.ds(8 * n, 8), :] = pltpu.pack_elementwise([kv[t2][0:8], kv[t2][8:16]], packed_dtype=BF)
        yield 100


def b_front_h(h_s, ht_s, hs, m):
    for tt in range(4):
        c0 = 512 * m + 128 * tt
        ht_s[pl.ds(c0 // 2, 64), :] = pltpu.bitcast(_bf(h_s[:, pl.ds(c0, 128)]).T, U32)
        yield 40
    hw = ht_s
    m16 = jnp.uint32(0xFFFF)
    mh = jnp.uint32(0xFFFF0000)
    for n in range(8):
        base = 256 * m + 32 * n
        A0 = hw[pl.ds(base + 0, 8, stride=2), :]
        B0 = hw[pl.ds(base + 16, 8, stride=2), :]
        A1 = hw[pl.ds(base + 1, 8, stride=2), :]
        B1 = hw[pl.ds(base + 17, 8, stride=2), :]
        P = [(A0 & m16) | (B0 << 16), (A0 >> 16) | (B0 & mh),
             (A1 & m16) | (B1 << 16), (A1 >> 16) | (B1 & mh)]
        for t2 in range(4):
            hs[t2, m, pl.ds(8 * n, 8), :] = P[t2]
        if n % 4 == 3:
            yield 48


def b_fwd(f_ref, xs, ax, j, dvec=None):
    CH = FWD_CH
    X = [_bf(xs[t2, j]) for t2 in range(4)]

    def finish(ch, A):
        for pp in range(CH // 16):
            p = ch * (CH // 16) + pp
            a = [(A[t2][16 * pp:16 * pp + 8], A[t2][16 * pp + 8:16 * pp + 16]) for t2 in range(4)]
            if dvec is not None:
                a[0] = (a[0][0] + dvec, a[0][1])
            Xk = _radix4(a)
            for k in range(4):
                ax[k, j, pl.ds(16 * p, 8), :] = Xk[k][0]
                ax[k, j, pl.ds(16 * p + 8, 8), :] = Xk[k][1]

    prev = None
    for ch in range(256 // CH):
        A = [_dot(_bf(f_ref[t2, pl.ds(ch * CH // 2, CH // 2), :]), X[t2]) for t2 in range(4)]
        if prev is not None:
            finish(*prev)
        prev = (ch, A)
        yield CH * 5
    finish(*prev)
    yield CH


def _call(fn):
    if fn is not None:
        fn()
    yield 0


def b_first(k_s, v_s, h_s, sk, dvec, ht_s, xs, hs, f_ref, ax, ah, wait_x=None, wait_h=None):
    fx = lambda j: b_front_x(k_s, v_s, sk, xs, j)
    fh = lambda m: b_front_h(h_s, ht_s, hs, m)
    dx = lambda j: b_fwd(f_ref, xs, ax, j)
    dh = lambda m: b_fwd(f_ref, hs, ah, m, dvec if m == 0 else None)
    for g in (_call(wait_x), fx(0), fx(1), dx(0), fx(2), dx(1), fx(3), dx(2), _call(wait_h), fh(0), dx(3), fh(1),
              dh(0), fh(2), dh(1), fh(3), dh(2), dh(3)):
        yield from g


BF_TOT = 32 * 100 + 4 * (160 + 96) + 8 * (256 * 5 + FWD_CH)


def b_mid(ax, ah, vs):
    for p in range(16):
        pos = p < 8
        r_re = pl.ds(16 * p, 8)
        r_im = pl.ds(16 * p + 8, 8)
        Zp = None
        for i in range(4):
            Z = []
            for k in range(4):
                wr = None
                wi = None
                for j in range(i + 1):
                    xr, xi = ax[k, j, r_re, :], ax[k, j, r_im, :]
                    gr, gi = ah[k, i - j, r_re, :], ah[k, i - j, r_im, :]
                    pr = xr * gr - xi * gi
                    pi = xr * gi + xi * gr
                    wr = pr if wr is None else wr + pr
                    wi = pi if wi is None else wi + pi
                Z.append((wr, wi))
            if Zp is None:
                W = Z
            elif pos:
                W = [(Z[k][0] - Zp[k][1], Z[k][1] + Zp[k][0]) for k in range(4)]
            else:
                W = [(Z[k][0] + Zp[k][1], Z[k][1] - Zp[k][0]) for k in range(4)]
            Zp = Z
            V = _iradix4(W)
            for t2 in range(4):
                vs[t2, i, pl.ds(8 * p, 8), :] = pltpu.pack_elementwise([V[t2][0], V[t2][1]], packed_dtype=BF)
            yield 40 + 32 * (i + 1) + (8 if i else 0)


def b_back(vs, finv_ref, q_s, o_s, blocks=range(4)):
    qw = q_s.bitcast(U32)
    ow = o_s.bitcast(U32)
    CH = BACK_CH

    def finish(base, y):
        E = qw[pl.ds(base, CH, stride=2), :]
        ow[pl.ds(base, CH, stride=2), :] = pltpu.pack_elementwise(
            [_lo(E) * y[0], _hi(E) * y[1]], packed_dtype=BF)

    prev = None
    for i in blocks:
        for hf in range(2):
            Vt = [_bf(vs[2 * hf + e, i]) for e in range(2)]
            for ch in range(128 // CH):
                y = [_dot(_bf(finv_ref[2 * hf + e, pl.ds(ch * CH // 2, CH // 2), :]), Vt[e]) for e in range(2)]
                if prev is not None:
                    finish(*prev)
                prev = (256 * i + 2 * CH * ch + hf, y)
                yield CH * 5
    finish(*prev)
    yield CH


def _p_dots(p_acc, g, pkt, xt, first=False):
    for n in range(4):
        cs = pl.ds(256 * n, 256)
        d = _dot(pkt, xt[:, 256 * n:256 * (n + 1)])
        if first:
            p_acc[g, :, cs] = d
        else:
            p_acc[g, :, cs] += d
        yield 128


def _k_finish(z_acc, col, kf0, kf1):
    pk = jnp.concatenate([_phi(kf0), _phi(kf1)], axis=0)
    z_acc[:, pl.ds(col, 128)] += jnp.sum(pk.reshape(R // 8, 8, 128), axis=0)
    return pk.astype(BF).T


def a_phase1(x_s, w_s, r0, p_acc, z_acc, pb_s):
    rw = pl.multiple_of(r0 // 2, R // 2)
    xprev = lambda: _bf(x_s[pl.ds(pl.multiple_of(rw - R // 2, R // 2), R // 2), :])
    xfull = lambda: _bf(x_s[pl.ds(rw, R // 2), :])
    pend = None
    pend2 = None
    for g in range(8):
        wk = lambda: _bf(w_s[:, pl.ds(1024 + 128 * g, 128)])
        kf0 = _dot(_bf(x_s[pl.ds(rw, MA // 2), :]), wk())
        yield 256
        if g == 0:
            yield from _p_dots(p_acc, 7, _bf(pb_s[...]), xprev())
        if pend is not None:
            pend2 = (pend[0], _k_finish(z_acc, 128 * pend[0], pend[1], pend[2]))
        kf1 = _dot(_bf(x_s[pl.ds(pl.multiple_of(rw + MA // 2, MA // 2), MA // 2), :]), wk())
        yield 256
        if pend2 is not None:
            yield from _p_dots(p_acc, pend2[0], pend2[1], xfull())
            pend2 = None
        pend = (g, kf0, kf1)
    pb_s[...] = pltpu.bitcast(_k_finish(z_acc, 128 * pend[0], pend[1], pend[2]), U32)
    yield 16


A1_TOT = 8 * 1024 + 16


def a_boundary_prep(z_acc, zt_s):
    z = jnp.sum(z_acc[...], axis=0, keepdims=True)
    zt_s[...] = jnp.broadcast_to(z, (8, D))


def a_boundary(p_acc, w_s, wo_s, m_s):
    ri = lax.broadcasted_iota(jnp.int32, (128, 128), 0) // 32
    ci = lax.broadcasted_iota(jnp.int32, (128, 128), 1) // 32
    same = ri == ci

    pb = [None] * 8
    kv = [None] * 8
    kvb = [None] * 8

    def prep(g):
        if g < 8:
            pb[g] = p_acc[g].astype(BF)

    def kv_dot(g):
        kv[g] = _dot(pb[g], _bf(w_s[:, pl.ds(2048 + 128 * g, 128)]))

    def mask(g):
        kvb[g] = jnp.where(same, kv[g], 0.0).astype(BF)

    def m_dots(g):
        m_s[pl.ds(64 * g, 64), :] = _pk(_dot(kvb[g], _bf(wo_s[pl.ds(64 * g, 64), :])))
        yield 256

    prep(0)
    prep(1)
    yield 32
    for t in range(10):
        if t < 8:
            kv_dot(t)
            prep(t + 2)
        if 1 <= t <= 8:
            mask(t - 1)
        if t < 8:
            yield 256
        if t >= 2:
            yield from m_dots(t - 2)


def _head_normalize_rows(rows, z):
    lane = lax.broadcasted_iota(jnp.int32, (8, 128), 1)
    cur = [r * z for r in rows]
    pos = [0] * len(cur)
    groups = [[j] for j in range(len(cur))]
    sh = 16
    while len(cur) > 1:
        nxt = []
        ng = []
        upper = (lane & sh) != 0
        for a in range(0, len(cur), 2):
            u = cur[a] + pltpu.roll(cur[a], sh, 1)
            v = cur[a + 1] + pltpu.roll(cur[a + 1], 128 - sh, 1)
            nxt.append(jnp.where(upper, u, v))
            for j in groups[a]:
                pos[j] |= sh
            ng.append(groups[a] + groups[a + 1])
        cur = nxt
        groups = ng
        sh //= 2
    m = cur[0]
    fill = 0
    while sh >= 1:
        m = m + pltpu.roll(m, sh, 1)
        fill |= sh
        sh //= 2
    r = pl.reciprocal(m + 1e-6, approx=True)
    return [rows[j] * jnp.take_along_axis(r, (lane & ~31) | (pos[j] | fill), axis=1) for j in range(len(rows))]


def _head_normalize(pq, z):
    rows = [pq[8 * j:8 * j + 8] for j in range(MA // 8)]
    out = []
    for a in range(0, len(rows), NORM_GROUP):
        out += _head_normalize_rows(rows[a:a + NORM_GROUP], z)
    return jnp.concatenate(out, axis=0)


def a_phase2(x_s, w_s, r0, zr_s, m_s, wg_s, oa_s):
    def fin(g, mc, qf):
        wg_s[mc, :, pl.ds(128 * g, 128)] = _pk(_head_normalize(_phi(qf), zr_s[:, pl.ds(128 * g, 128)]))

    def out_dot(mc, n):
        wg = _bf(wg_s[mc])
        oa_s[pl.ds(mc * (MA // 2), MA // 2), pl.ds(128 * n, 128)] = _pk(_dot(wg, _bf(m_s[:, pl.ds(128 * n, 128)])))

    p1 = None
    nmc = R // MA
    for mc in range(nmc):
        rw = pl.multiple_of(r0 // 2 + mc * (MA // 2), MA // 2)
        for g in range(8):
            xt = _bf(x_s[pl.ds(rw, MA // 2), :])
            qf = _dot(xt, _bf(w_s[:, pl.ds(128 * g, 128)]))
            if p1 is not None:
                fin(*p1)
            p1 = (g, mc, qf)
            yield A2_WQ
            if mc > 0 and g >= 3:
                out_dot(mc - 1, g - 3)
                yield A2_WO
    out_dot(nmc - 2, 5)
    fin(*p1)
    yield A2_WO
    out_dot(nmc - 2, 6)
    yield A2_WO
    out_dot(nmc - 2, 7)
    yield A2_WO
    for n in range(8):
        out_dot(nmc - 1, n)
        yield A2_WO


A2_TOT = 16 * (A2_WQ + A2_WO)


def _interleave(a_items, b_items, a_tot, b_tot, lead=0.0, tail=0.0):
    a_done = 0.0
    b_done = 0.0
    a_alive = True
    b_alive = True
    while a_alive or b_alive:
        fa = (a_done / a_tot - lead) / (1.0 - lead - tail)
        fb = b_done / b_tot
        if b_alive and (not a_alive or fb < fa):
            try:
                b_done += next(b_items)
            except StopIteration:
                b_alive = False
        else:
            try:
                a_done += next(a_items)
            except StopIteration:
                a_alive = False


def _chain(*gens):
    for g in gens:
        yield from g


BM_TOT = 16 * (160 + 320 + 24)
BK_TOT = 8 * 128 * 5 + BACK_CH
STAGE2_AT = 3
A1F_LEAD = 0.2
BD_TOT = 8 * 512 + 32


def _run(gen):
    for _ in gen:
        pass


def a_start(x_s, w_s, p_acc, z_acc, pb_s, wait_chunk):
    pb_s[...] = jnp.zeros_like(pb_s)
    p_acc[7] = jnp.zeros((128, D), F32)

    def body(g, carry):
        wait_chunk(g)
        ck = pl.multiple_of(1024 + 128 * g, 128)
        col = pl.multiple_of(128 * g, 128)
        kf0 = _dot(_bf(x_s[pl.ds(0, MA // 2), :]), _bf(w_s[:, pl.ds(ck, 128)]))
        kf1 = _dot(_bf(x_s[pl.ds(MA // 2, MA // 2), :]), _bf(w_s[:, pl.ds(ck, 128)]))
        prev = _bf(pb_s[...])
        cur = _k_finish(z_acc, col, kf0, kf1)
        _run(_p_dots(p_acc, jnp.maximum(g - 1, 0), prev, _bf(x_s[pl.ds(0, R // 2), :]), first=True))
        pb_s[...] = pltpu.bitcast(cur, U32)
        return carry

    lax.fori_loop(0, 8, body, 0)


def kernel(x_hbm, w_hbm, wo_hbm, q_hbm, k_hbm, v_hbm, h_hbm, skT_hbm, d_hbm, f_hbm, finv_hbm, o_hbm,
           x_s, w_s, wo_s, m_s, p_acc, z_acc, zt_s, wg_s, oa_s,
           q_s, k_s, v_s, h_s, o_s, ht_s, xs, hs, ax, ah, vs, d_s,
           skT_ref, d_ref, f_ref, finv_ref, pb_s, flag_s,
           sem_x, sem_w, sem_wc, sem_c, sem_b, sem_ob, sem_oa):
    def x_cp(i):
        return pltpu.make_async_copy(x_hbm.at[0, pl.ds(i * R, R), :],
                                     x_s.bitcast(BF).at[pl.ds(i * R, R), :], sem_x.at[i])

    def wc_cp(g):
        col = pl.multiple_of(1024 + 128 * g, 128)
        return pltpu.make_async_copy(w_hbm.at[:, pl.ds(col, 128)],
                                     w_s.bitcast(BF).at[:, pl.ds(col, 128)], sem_wc.at[g])

    wv_cp = pltpu.make_async_copy(w_hbm.at[:, pl.ds(2048, 1024)], w_s.bitcast(BF).at[:, pl.ds(2048, 1024)],
                                  sem_w.at[2])

    wq_cp = pltpu.make_async_copy(w_hbm.at[:, pl.ds(0, 1024)], w_s.bitcast(BF).at[:, pl.ds(0, 1024)], sem_w.at[0])
    wo_cp = pltpu.make_async_copy(wo_hbm, wo_s.bitcast(BF), sem_w.at[1])
    c_cps = [pltpu.make_async_copy(skT_hbm, skT_ref, sem_c.at[0]),
             pltpu.make_async_copy(d_hbm, d_ref, sem_c.at[1]),
             pltpu.make_async_copy(f_hbm, f_ref, sem_c.at[2]),
             pltpu.make_async_copy(finv_hbm, finv_ref, sem_c.at[3])]

    def f_in(c):
        col = pl.multiple_of(c * C, C)
        return [
            pltpu.make_async_copy(k_hbm.at[0, :, pl.ds(col, C)], k_s.at[c % 2, pl.ds(16, S), :], sem_b.at[4 * (c % 2) + 0]),
            pltpu.make_async_copy(v_hbm.at[0, :, pl.ds(col, C)], v_s.at[c % 2, pl.ds(0, S), :], sem_b.at[4 * (c % 2) + 1]),
            pltpu.make_async_copy(h_hbm.at[pl.ds(col, C), :], h_s.bitcast(BF).at[c % 2], sem_b.at[4 * (c % 2) + 2]),
        ]

    def q_cp(c):
        col = pl.multiple_of(c * C, C)
        return pltpu.make_async_copy(q_hbm.at[0, :, pl.ds(col, C)], q_s.at[c % 2, pl.ds(0, S), :],
                                     sem_b.at[4 * (c % 2) + 3])

    def ob_cp(c):
        col = pl.multiple_of(D + c * C, C)
        return pltpu.make_async_copy(o_s.at[pl.ds(0, S), :], o_hbm.at[0, :, pl.ds(col, C)], sem_ob.at[0])

    def ob_last_cp(i):
        return pltpu.make_async_copy(o_s.at[pl.ds(512 * i, 512), :],
                                     o_hbm.at[0, pl.ds(512 * i, 512), pl.ds(D + (NT - 1) * C, C)], sem_ob.at[1 + i])

    def oa_cp(i, slot):
        r = pl.multiple_of(i * R, R)
        return pltpu.make_async_copy(oa_s.bitcast(BF).at[slot], o_hbm.at[0, pl.ds(r, R), pl.ds(0, D)], sem_oa.at[slot])

    def gen_f(c, wait_x=None, wait_h=None):
        col = pl.multiple_of(c * C, C)
        sk = [skT_ref[pl.ds(i, 1), pl.ds(col, C)].astype(F32) for i in range(4)]
        dvec = d_s[:, pl.ds(col, C)]
        sl = c % 2
        return b_first(k_s.at[sl], v_s.at[sl], h_s.at[sl], sk, dvec, ht_s, xs, hs, f_ref, ax, ah, wait_x, wait_h)

    def gen_m():
        return b_mid(ax, ah, vs)

    def gen_k(c, blocks=range(4)):
        return b_back(vs, finv_ref, q_s.at[c % 2], o_s, blocks)

    def a1(s):
        return a_phase1(x_s, w_s, pl.multiple_of(s * R, R), p_acc, z_acc, pb_s)

    def a2(s, slot):
        return a_phase2(x_s, w_s, pl.multiple_of(s * R, R), zt_s, m_s, wg_s, oa_s.at[slot])

    def post_f(c):
        @pl.when(c + 1 < NT)
        def _():
            q_cp(c + 1).start()

        @pl.when(c + 2 < NT)
        def _():
            for cp in f_in(c + 2):
                cp.start()

    def pre_kf(c):
        q_cp(c).wait()

        @pl.when(c + 1 < NT)
        def _():
            for cp in f_in(c + 1):
                cp.wait()

        @pl.when(c >= 1)
        def _():
            ob_cp(c - 1).wait()

    flag_s[0] = 1
    x_cp(0).start()
    for g in range(8):
        wc_cp(g).start()
    z_acc[...] = jnp.zeros_like(z_acc)
    for sl in range(2):
        k_s[sl, pl.ds(0, 16), :] = jnp.zeros((16, C), BF)
    with jax.named_scope("w_x0"):
        x_cp(0).wait()

    def wait_chunk(g):
        wc_cp(g).wait()

        @pl.when(g == STAGE2_AT)
        def _():
            x_cp(1).start()
            for cp in c_cps:
                cp.start()
            for cp in f_in(0):
                cp.start()

    with jax.named_scope("s0"):
        a_start(x_s, w_s, p_acc, z_acc, pb_s, wait_chunk)
    x_cp(2).start()
    q_cp(0).start()
    for cp in f_in(1):
        cp.start()
    with jax.named_scope("w_c"):
        x_cp(1).wait()
        for cp in c_cps[:3]:
            cp.wait()
    d_s[...] = d_ref[...].reshape(1, D).astype(F32)

    def wait_kv0():
        for cp in f_in(0)[:2]:
            cp.wait()

    def wait_h0():
        f_in(0)[2].wait()

    with jax.named_scope("a1f"):
        _interleave(a1(1), gen_f(0, wait_kv0, wait_h0), A1_TOT, BF_TOT, lead=A1F_LEAD)
    post_f(0)
    for i in range(3, NR):
        x_cp(i).start()
    wq_cp.start()
    wv_cp.start()
    wo_cp.start()
    c_cps[3].wait()

    def phase1_body(s, carry):
        c = (s - 2) // 2
        x_cp(s).wait()

        @pl.when(s % 2 == 0)
        def _():
            with jax.named_scope("a1m"):
                _interleave(a1(s), gen_m(), A1_TOT, BM_TOT)

        @pl.when(s % 2 == 1)
        def _():
            pre_kf(c)

        @pl.when(s % 2 == 1)
        def _():
            with jax.named_scope("a1kf"):
                _interleave(a1(s), _chain(gen_k(c), gen_f(c + 1)), A1_TOT, BK_TOT + BF_TOT)

        @pl.when(flag_s[0] + s % 2 == 2)
        def _():
            ob_cp(c).start()
            post_f(c + 1)
        return carry

    lax.fori_loop(2, 8, phase1_body, 0)

    wq_cp.wait()
    wv_cp.wait()
    wo_cp.wait()
    with jax.named_scope("bdprep"):
        _run(_p_dots(p_acc, 7, _bf(pb_s[...]), _bf(x_s[pl.ds((S - R) // 2, R // 2), :])))
        a_boundary_prep(z_acc, zt_s)

    @pl.when(flag_s[0] == 1)
    def _():
        with jax.named_scope("bd"):
            _interleave(a_boundary(p_acc, w_s, wo_s, m_s), gen_m(), BD_TOT, BM_TOT)


    def phase2_body(s, carry):
        c = 3 + s // 2

        @pl.when(s >= 2)
        def _():
            oa_cp(s - 2, s % 2).wait()

        @pl.when(s % 2 == 0)
        def _():
            pre_kf(c)

        @pl.when(s % 2 == 0)
        def _():
            with jax.named_scope("a2kf"):
                _interleave(a2(s, 0), _chain(gen_k(c), gen_f(c + 1)), A2_TOT, BK_TOT + BF_TOT)

        @pl.when(s % 2 == 1)
        def _():
            with jax.named_scope("a2m"):
                _interleave(a2(s, 1), gen_m(), A2_TOT, BM_TOT)

        @pl.when(flag_s[0] + s % 2 == 1)
        def _():
            oa_cp(s, 0).start()
            ob_cp(c).start()
            post_f(c + 1)

        @pl.when(flag_s[0] + s % 2 == 2)
        def _():
            oa_cp(s, 1).start()
        return carry

    lax.fori_loop(0, 8, phase2_body, 0)
    q_cp(7).wait()
    ob_cp(6).wait()

    with jax.named_scope("lastk"):
        for i in range(4):
            _run(gen_k(NT - 1, [i]))
            ob_last_cp(i).start()
    with jax.named_scope("endwait"):
        oa_cp(6, 0).wait()
        oa_cp(7, 1).wait()
        for i in range(4):
            ob_last_cp(i).wait()


@jax.jit
def pallas_concat_heads__linear_attn_block__ssm_conv_h3__prompt_kernel(A_x, A_wqkv, A_wo, B_q, B_k, B_v, B_shift_k, B_ssm_k, B_ssm_D):
    any_spec = pl.BlockSpec(memory_space=pl.ANY)
    return pl.pallas_call(
        kernel,
        in_specs=[any_spec] * 11,
        out_specs=any_spec,
        out_shape=jax.ShapeDtypeStruct((1, S, 2 * D), BF),
        scratch_shapes=[
            pltpu.VMEM((S // 2, D), U32),
            pltpu.VMEM((D // 2, 3 * D), U32),
            pltpu.VMEM((D // 2, D), U32),
            pltpu.VMEM((D // 2, D), U32),
            pltpu.VMEM((8, 128, D), F32),
            pltpu.VMEM((8, D), F32),
            pltpu.VMEM((8, D), F32),
            pltpu.VMEM((R // MA, MA // 2, D), U32),
            pltpu.VMEM((2, R // 2, D), U32),
            pltpu.VMEM((2, S + 16, C), BF),
            pltpu.VMEM((2, S + 32, C), BF),
            pltpu.VMEM((2, S + 16, C), BF),
            pltpu.VMEM((2, C // 2, S), U32),
            pltpu.VMEM((S + 16, C), BF),
            pltpu.VMEM((S // 2 + 8, C), U32),
            pltpu.VMEM((4, 4, 64, 128), U32),
            pltpu.VMEM((4, 4, 64, 128), U32),
            pltpu.VMEM((4, 4, 256, 128), F32),
            pltpu.VMEM((4, 4, 256, 128), F32),
            pltpu.VMEM((4, 4, 128, 128), U32),
            pltpu.VMEM((1, D), F32),
            pltpu.VMEM((4, D), BF),
            pltpu.VMEM((D,), BF),
            pltpu.VMEM((4, 128, 128), U32),
            pltpu.VMEM((4, 64, 256), U32),
            pltpu.VMEM((64, R), U32),
            pltpu.SMEM((1,), jnp.int32),
            pltpu.SemaphoreType.DMA((NR,)),
            pltpu.SemaphoreType.DMA((3,)),
            pltpu.SemaphoreType.DMA((8,)),
            pltpu.SemaphoreType.DMA((4,)),
            pltpu.SemaphoreType.DMA((8,)),
            pltpu.SemaphoreType.DMA((5,)),
            pltpu.SemaphoreType.DMA((2,)),
        ],
        compiler_params=pltpu.CompilerParams(vmem_limit_bytes=100 * 1024 * 1024, disable_bounds_checks=True, disable_semaphore_checks=True),
        name="fused",
    )(A_x, A_wqkv, A_wo, B_q, B_k, B_v, B_ssm_k, B_shift_k.T, B_ssm_D,
      jnp.asarray(_F_PK), jnp.asarray(_FINV_PK))
```

```python
import numpy as np
import jax
import jax.numpy as jnp
from jax import lax
from jax.experimental import pallas as pl
from jax.experimental.pallas import tpu as pltpu

S, D = 2048, 1024
C = 128
NT = D // C
MF = 1024
R = 256
NR = S // R
MA = 128
BF = jnp.bfloat16
F32 = jnp.float32
U32 = jnp.uint32

A2_WQ = 256
A2_WO = 256
NORM_GROUP = 16
FWD_CH = 128
BACK_CH = 64


def _make_consts():
    p = np.arange(16)[:, None]
    s = np.arange(8)[None, :]
    k1 = np.where(p < 8, 2 * (8 * p + s), 2 * (8 * (p - 8) + s) + 1)
    t1 = np.arange(128)
    F = np.zeros((4, 256, 128), np.float64)
    for t2 in range(4):
        th = 2 * np.pi * (4 * t1[None, None, :] + t2) * (k1[:, :, None] + 0.5) / MF
        F[t2] = np.stack([np.cos(th), -np.sin(th)], axis=1).reshape(256, 128)
    Finv = np.transpose(F.reshape(4, 16, 2, 8, 128), (0, 4, 1, 3, 2)).reshape(4, 128, 256) * (2.0 / MF)
    c = np.arange(128)
    perm = 16 * (c // 16) + 8 * ((c & 1)) + (c % 16) // 2
    F = F[:, :, perm]
    return F.astype(np.float32), Finv.astype(np.float32)


def _pack_rows(a):
    a = np.ascontiguousarray(a, np.float32)
    u = a.view(np.uint32)
    b = ((u + 0x7FFF + ((u >> 16) & 1)) >> 16).astype(np.uint32)
    return (b[..., 0::2, :] | (b[..., 1::2, :] << 16)).astype(np.uint32)


_F_NP, _FINV_NP = _make_consts()
_F_PK = _pack_rows(_F_NP)
_FINV_PK = _pack_rows(_FINV_NP)


def _lo(w):
    return pltpu.bitcast(w << 16, F32)


def _hi(w):
    return pltpu.bitcast(w & jnp.uint32(0xFFFF0000), F32)


def _bf(w):
    return pltpu.bitcast(w, BF)


def _pk(v):
    return pltpu.bitcast(v.astype(BF), U32)


def _dot(a, b):
    return jnp.dot(a, b, preferred_element_type=F32)


def _phi(t):
    return jnp.where(t > 0, t + 1.0, jnp.exp(t)) + 1e-6


def _radix4(A):
    (r0, i0), (r1, i1), (r2, i2), (r3, i3) = A
    a0r, a0i = r0 + r2, i0 + i2
    a1r, a1i = r0 - r2, i0 - i2
    b0r, b0i = r1 + r3, i1 + i3
    b1r, b1i = r1 - r3, i1 - i3
    return [(a0r + b0r, a0i + b0i), (a1r + b1i, a1i - b1r),
            (a0r - b0r, a0i - b0i), (a1r - b1i, a1i + b1r)]


def _iradix4(W):
    (r0, i0), (r1, i1), (r2, i2), (r3, i3) = W
    c0r, c0i = r0 + r2, i0 + i2
    c1r, c1i = r0 - r2, i0 - i2
    d0r, d0i = r1 + r3, i1 + i3
    d1r, d1i = r1 - r3, i1 - i3
    return [(c0r + d0r, c0i + d0i), (c1r - d1i, c1i + d1r),
            (c0r - d0r, c0i - d0i), (c1r + d1i, c1i - d1r)]


def b_front_x(k_s, v_s, sk, xs, j):
    kw = k_s.bitcast(U32)
    vw = v_s.bitcast(U32)
    s0, s1, s2, s3 = sk
    for n in range(8):
        t0 = 128 * j + 16 * n
        base = 8 + 2 * t0
        E = kw[pl.ds(base, 16, stride=2), :]
        O = kw[pl.ds(base + 1, 16, stride=2), :]
        Ep = kw[pl.ds(base - 2, 16, stride=2), :]
        Op = kw[pl.ds(base - 1, 16, stride=2), :]
        k0, k1, k2, k3 = _lo(E), _hi(E), _lo(O), _hi(O)
        k1p, k2p, k3p = _hi(Ep), _lo(Op), _hi(Op)
        Ev = vw[pl.ds(2 * t0, 16, stride=2), :]
        Ov = vw[pl.ds(2 * t0 + 1, 16, stride=2), :]
        ks0 = s0 * k0 + s1 * k3p + s2 * k2p + s3 * k1p
        ks1 = s0 * k1 + s1 * k0 + s2 * k3p + s3 * k2p
        ks2 = s0 * k2 + s1 * k1 + s2 * k0 + s3 * k3p
        ks3 = s0 * k3 + s1 * k2 + s2 * k1 + s3 * k0
        kv = [ks0 * _lo(Ev), ks1 * _hi(Ev), ks2 * _lo(Ov), ks3 * _hi(Ov)]
        for t2 in range(4):
            xs[t2, j, pl.ds(8 * n, 8), :] = pltpu.pack_elementwise([kv[t2][0:8], kv[t2][8:16]], packed_dtype=BF)
        yield 100


def b_front_h(h_s, ht_s, hs, m):
    for tt in range(4):
        c0 = 512 * m + 128 * tt
        ht_s[pl.ds(c0 // 2, 64), :] = pltpu.bitcast(_bf(h_s[:, pl.ds(c0, 128)]).T, U32)
        yield 40
    hw = ht_s
    m16 = jnp.uint32(0xFFFF)
    mh = jnp.uint32(0xFFFF0000)
    for n in range(8):
        base = 256 * m + 32 * n
        A0 = hw[pl.ds(base + 0, 8, stride=2), :]
        B0 = hw[pl.ds(base + 16, 8, stride=2), :]
        A1 = hw[pl.ds(base + 1, 8, stride=2), :]
        B1 = hw[pl.ds(base + 17, 8, stride=2), :]
        P = [(A0 & m16) | (B0 << 16), (A0 >> 16) | (B0 & mh),
             (A1 & m16) | (B1 << 16), (A1 >> 16) | (B1 & mh)]
        for t2 in range(4):
            hs[t2, m, pl.ds(8 * n, 8), :] = P[t2]
        if n % 4 == 3:
            yield 48


def b_fwd(f_ref, xs, ax, j, dvec=None):
    CH = FWD_CH
    X = [_bf(xs[t2, j]) for t2 in range(4)]

    def finish(ch, A):
        for pp in range(CH // 16):
            p = ch * (CH // 16) + pp
            a = [(A[t2][16 * pp:16 * pp + 8], A[t2][16 * pp + 8:16 * pp + 16]) for t2 in range(4)]
            if dvec is not None:
                a[0] = (a[0][0] + dvec, a[0][1])
            Xk = _radix4(a)
            for k in range(4):
                ax[k, j, pl.ds(16 * p, 8), :] = Xk[k][0]
                ax[k, j, pl.ds(16 * p + 8, 8), :] = Xk[k][1]

    prev = None
    for ch in range(256 // CH):
        A = [_dot(_bf(f_ref[t2, pl.ds(ch * CH // 2, CH // 2), :]), X[t2]) for t2 in range(4)]
        if prev is not None:
            finish(*prev)
        prev = (ch, A)
        yield CH * 5
    finish(*prev)
    yield CH


def b_first(k_s, v_s, h_s, sk, dvec, ht_s, xs, hs, f_ref, ax, ah, part=None):
    fx = lambda j: b_front_x(k_s, v_s, sk, xs, j)
    fh = lambda m: b_front_h(h_s, ht_s, hs, m)
    dx = lambda j: b_fwd(f_ref, xs, ax, j)
    dh = lambda m: b_fwd(f_ref, hs, ah, m, dvec if m == 0 else None)
    if part == "x":
        seq = (fx(0), fx(1), dx(0), fx(2), dx(1), fx(3), dx(2), dx(3))
    elif part == "h":
        seq = (fh(0), fh(1), dh(0), fh(2), dh(1), fh(3), dh(2), dh(3))
    else:
        seq = (fx(0), fx(1), dx(0), fx(2), dx(1), fx(3), dx(2), fh(0), dx(3), fh(1),
               dh(0), fh(2), dh(1), fh(3), dh(2), dh(3))
    for g in seq:
        yield from g


BF_TOT = 32 * 100 + 4 * (160 + 96) + 8 * (256 * 5 + FWD_CH)


def b_mid(ax, ah, vs):
    for p in range(16):
        pos = p < 8
        r_re = pl.ds(16 * p, 8)
        r_im = pl.ds(16 * p + 8, 8)
        Zp = None
        for i in range(4):
            Z = []
            for k in range(4):
                wr = None
                wi = None
                for j in range(i + 1):
                    xr, xi = ax[k, j, r_re, :], ax[k, j, r_im, :]
                    gr, gi = ah[k, i - j, r_re, :], ah[k, i - j, r_im, :]
                    pr = xr * gr - xi * gi
                    pi = xr * gi + xi * gr
                    wr = pr if wr is None else wr + pr
                    wi = pi if wi is None else wi + pi
                Z.append((wr, wi))
            if Zp is None:
                W = Z
            elif pos:
                W = [(Z[k][0] - Zp[k][1], Z[k][1] + Zp[k][0]) for k in range(4)]
            else:
                W = [(Z[k][0] + Zp[k][1], Z[k][1] - Zp[k][0]) for k in range(4)]
            Zp = Z
            V = _iradix4(W)
            for t2 in range(4):
                vs[t2, i, pl.ds(8 * p, 8), :] = pltpu.pack_elementwise([V[t2][0], V[t2][1]], packed_dtype=BF)
            yield 40 + 32 * (i + 1) + (8 if i else 0)


def b_back(vs, finv_ref, q_s, o_s, blocks=range(4)):
    qw = q_s.bitcast(U32)
    ow = o_s.bitcast(U32)
    CH = BACK_CH

    def finish(base, y):
        E = qw[pl.ds(base, CH, stride=2), :]
        ow[pl.ds(base, CH, stride=2), :] = pltpu.pack_elementwise(
            [_lo(E) * y[0], _hi(E) * y[1]], packed_dtype=BF)

    prev = None
    for i in blocks:
        for hf in range(2):
            Vt = [_bf(vs[2 * hf + e, i]) for e in range(2)]
            for ch in range(128 // CH):
                y = [_dot(_bf(finv_ref[2 * hf + e, pl.ds(ch * CH // 2, CH // 2), :]), Vt[e]) for e in range(2)]
                if prev is not None:
                    finish(*prev)
                prev = (256 * i + 2 * CH * ch + hf, y)
                yield CH * 5
    finish(*prev)
    yield CH


def _p_dots(p_acc, g, pkt, xt, first=False):
    for n in range(4):
        cs = pl.ds(256 * n, 256)
        d = _dot(pkt, xt[:, 256 * n:256 * (n + 1)])
        if first:
            p_acc[g, :, cs] = d
        else:
            p_acc[g, :, cs] += d
        yield 128


def _k_finish(z_acc, col, kf0, kf1):
    pk = jnp.concatenate([_phi(kf0), _phi(kf1)], axis=0)
    z_acc[:, pl.ds(col, 128)] += jnp.sum(pk.reshape(R // 8, 8, 128), axis=0)
    return pk.astype(BF).T


def a_phase1(x_s, w_s, r0, p_acc, z_acc, pb_s, wait_chunk=None):
    rw = r0
    xprev = lambda: _bf(x_s[pl.ds(pl.multiple_of(rw - R // 2, R // 2), R // 2), :])
    xfull = lambda: _bf(x_s[pl.ds(rw, R // 2), :])
    pend = None
    pend2 = None
    first = wait_chunk is not None
    for g in range(8):
        if first:
            wait_chunk(g)
        wk = lambda: _bf(w_s[:, pl.ds(1024 + 128 * g, 128)])
        kf0 = _dot(_bf(x_s[pl.ds(rw, MA // 2), :]), wk())
        yield 256
        if g == 0 and not first:
            yield from _p_dots(p_acc, 7, _bf(pb_s[...]), xprev())
        if pend is not None:
            pend2 = (pend[0], _k_finish(z_acc, 128 * pend[0], pend[1], pend[2]))
        kf1 = _dot(_bf(x_s[pl.ds(pl.multiple_of(rw + MA // 2, MA // 2), MA // 2), :]), wk())
        yield 256
        if pend2 is not None:
            yield from _p_dots(p_acc, pend2[0], pend2[1], xfull(), first)
            pend2 = None
        pend = (g, kf0, kf1)
    pb_s[...] = pltpu.bitcast(_k_finish(z_acc, 128 * pend[0], pend[1], pend[2]), U32)
    yield 16


A1_TOT = 8 * 1024 + 16


def a_boundary_prep(z_acc, zt_s):
    z = jnp.sum(z_acc[...], axis=0, keepdims=True)
    zt_s[...] = jnp.broadcast_to(z, (8, D))


def a_boundary(p_acc, w_s, wo_s, m_s):
    ri = lax.broadcasted_iota(jnp.int32, (128, 128), 0) // 32
    ci = lax.broadcasted_iota(jnp.int32, (128, 128), 1) // 32
    same = ri == ci

    pb = [None] * 8
    kv = [None] * 8
    kvb = [None] * 8

    def prep(g):
        if g < 8:
            pb[g] = p_acc[g].astype(BF)

    def kv_dot(g):
        kv[g] = _dot(pb[g], _bf(w_s[:, pl.ds(2048 + 128 * g, 128)]))

    def mask(g):
        kvb[g] = jnp.where(same, kv[g], 0.0).astype(BF)

    def m_dots(g):
        m_s[pl.ds(64 * g, 64), :] = _pk(_dot(kvb[g], _bf(wo_s[pl.ds(64 * g, 64), :])))
        yield 256

    prep(0)
    prep(1)
    yield 32
    for t in range(10):
        if t < 8:
            kv_dot(t)
            prep(t + 2)
        if 1 <= t <= 8:
            mask(t - 1)
        if t < 8:
            yield 256
        if t >= 2:
            yield from m_dots(t - 2)


def _head_normalize_rows(rows, z):
    lane = lax.broadcasted_iota(jnp.int32, (8, 128), 1)
    cur = [r * z for r in rows]
    pos = [0] * len(cur)
    groups = [[j] for j in range(len(cur))]
    sh = 16
    while len(cur) > 1:
        nxt = []
        ng = []
        upper = (lane & sh) != 0
        for a in range(0, len(cur), 2):
            u = cur[a] + pltpu.roll(cur[a], sh, 1)
            v = cur[a + 1] + pltpu.roll(cur[a + 1], 128 - sh, 1)
            nxt.append(jnp.where(upper, u, v))
            for j in groups[a]:
                pos[j] |= sh
            ng.append(groups[a] + groups[a + 1])
        cur = nxt
        groups = ng
        sh //= 2
    m = cur[0]
    fill = 0
    while sh >= 1:
        m = m + pltpu.roll(m, sh, 1)
        fill |= sh
        sh //= 2
    r = pl.reciprocal(m + 1e-6, approx=True)
    return [rows[j] * jnp.take_along_axis(r, (lane & ~31) | (pos[j] | fill), axis=1) for j in range(len(rows))]


def _head_normalize(pq, z):
    rows = [pq[8 * j:8 * j + 8] for j in range(MA // 8)]
    out = []
    for a in range(0, len(rows), NORM_GROUP):
        out += _head_normalize_rows(rows[a:a + NORM_GROUP], z)
    return jnp.concatenate(out, axis=0)


def a_phase2(x_s, w_s, r0, zr_s, m_s, wg_s, oa_s, part=None):
    def fin(g, mc, qf):
        wg_s[mc, :, pl.ds(128 * g, 128)] = _pk(_head_normalize(_phi(qf), zr_s[:, pl.ds(128 * g, 128)]))

    def out_dot(mc, n):
        wg = _bf(wg_s[mc])
        oa_s[pl.ds(mc * (MA // 2), MA // 2), pl.ds(128 * n, 128)] = _pk(_dot(wg, _bf(m_s[:, pl.ds(128 * n, 128)])))

    p1 = None
    nmc = R // MA
    if part == "tail":
        for n in range(8):
            out_dot(nmc - 1, n)
            yield A2_WO
        return
    for mc in range(nmc):
        rw = pl.multiple_of(r0 + mc * (MA // 2), MA // 2)
        for g in range(8):
            xt = _bf(x_s[pl.ds(rw, MA // 2), :])
            qf = _dot(xt, _bf(w_s[:, pl.ds(128 * g, 128)]))
            if p1 is not None:
                fin(*p1)
            p1 = (g, mc, qf)
            yield A2_WQ
            if mc > 0 and g >= 3:
                out_dot(mc - 1, g - 3)
                yield A2_WO
    out_dot(nmc - 2, 5)
    fin(*p1)
    yield A2_WO
    out_dot(nmc - 2, 6)
    yield A2_WO
    out_dot(nmc - 2, 7)
    yield A2_WO
    if part == "head":
        return
    for n in range(8):
        out_dot(nmc - 1, n)
        yield A2_WO


A2_TOT = 16 * (A2_WQ + A2_WO)


def _interleave(a_items, b_items, a_tot, b_tot, lead=0.0, tail=0.0):
    a_done = 0.0
    b_done = 0.0
    a_alive = True
    b_alive = True
    while a_alive or b_alive:
        fa = (a_done / a_tot - lead) / (1.0 - lead - tail)
        fb = b_done / b_tot
        if b_alive and (not a_alive or fb < fa):
            try:
                b_done += next(b_items)
            except StopIteration:
                b_alive = False
        else:
            try:
                a_done += next(a_items)
            except StopIteration:
                a_alive = False


def _chain(*gens):
    for g in gens:
        yield from g


BFX_TOT = 32 * 100 + 4 * (256 * 5 + FWD_CH)
BM_TOT = 16 * (160 + 320 + 24)
BK_TOT = 8 * 128 * 5 + BACK_CH
S0_WAITS = {0: (0,), 1: (1, 2), 3: (3, 4, 5), 6: (6, 7)}
S0_F_AT = 6
LAST_TAIL = 0.1
BD_TOT = 8 * 512 + 32


def _run(gen):
    for _ in gen:
        pass


def kernel(x_hbm, w_hbm, wo_hbm, q_hbm, k_hbm, v_hbm, h_hbm, skT_hbm, d_hbm, f_hbm, finv_hbm, o_hbm,
           x_s, w_s, wo_s, m_s, p_acc, z_acc, zt_s, wg_s, oa_s,
           q_s, k_s, v_s, h_s, o_s, ht_s, xs, hs, ax, ah, vs, d_s,
           skT_ref, d_ref, f_ref, finv_ref, pb_s, flag_s,
           sem_x, sem_w, sem_wc, sem_c, sem_b, sem_ob, sem_oa):
    def x_cp(i):
        return pltpu.make_async_copy(x_hbm.at[0, pl.ds(i * R, R), :],
                                     x_s.bitcast(BF).at[pl.ds(i * R, R), :], sem_x.at[i])

    def wc_cp(g):
        col = pl.multiple_of(1024 + 128 * g, 128)
        return pltpu.make_async_copy(w_hbm.at[:, pl.ds(col, 128)],
                                     w_s.bitcast(BF).at[:, pl.ds(col, 128)], sem_wc.at[g])

    wv_cp = pltpu.make_async_copy(w_hbm.at[:, pl.ds(2048, 1024)], w_s.bitcast(BF).at[:, pl.ds(2048, 1024)],
                                  sem_w.at[2])

    wq_cp = pltpu.make_async_copy(w_hbm.at[:, pl.ds(0, 1024)], w_s.bitcast(BF).at[:, pl.ds(0, 1024)], sem_w.at[0])
    wo_cp = pltpu.make_async_copy(wo_hbm, wo_s.bitcast(BF), sem_w.at[1])
    c_cps = [pltpu.make_async_copy(skT_hbm, skT_ref, sem_c.at[0]),
             pltpu.make_async_copy(d_hbm, d_ref, sem_c.at[1]),
             pltpu.make_async_copy(f_hbm, f_ref, sem_c.at[2]),
             pltpu.make_async_copy(finv_hbm, finv_ref, sem_c.at[3])]

    def f_in(c):
        col = pl.multiple_of(c * C, C)
        return [
            pltpu.make_async_copy(k_hbm.at[0, :, pl.ds(col, C)], k_s.at[(c & 1), pl.ds(16, S), :], sem_b.at[4 * ((c & 1)) + 0]),
            pltpu.make_async_copy(v_hbm.at[0, :, pl.ds(col, C)], v_s.at[(c & 1), pl.ds(0, S), :], sem_b.at[4 * ((c & 1)) + 1]),
            pltpu.make_async_copy(h_hbm.at[pl.ds(col, C), :], h_s.bitcast(BF).at[(c & 1)], sem_b.at[4 * ((c & 1)) + 2]),
        ]

    def q_cp(c):
        col = pl.multiple_of(c * C, C)
        return pltpu.make_async_copy(q_hbm.at[0, :, pl.ds(col, C)], q_s.at[(c & 1), pl.ds(0, S), :],
                                     sem_b.at[4 * ((c & 1)) + 3])

    def ob_cp(c):
        col = pl.multiple_of(D + c * C, C)
        return pltpu.make_async_copy(o_s.at[pl.ds(0, S), :], o_hbm.at[0, :, pl.ds(col, C)], sem_ob.at[0])

    def ob_last_cp(i):
        return pltpu.make_async_copy(o_s.at[pl.ds(512 * i, 512), :],
                                     o_hbm.at[0, pl.ds(512 * i, 512), pl.ds(D + (NT - 1) * C, C)], sem_ob.at[1 + i])

    def oa_cp(i, slot):
        r = pl.multiple_of(i * R, R)
        return pltpu.make_async_copy(oa_s.bitcast(BF).at[slot], o_hbm.at[0, pl.ds(r, R), pl.ds(0, D)], sem_oa.at[slot])

    def gen_f(c, wait=None, part=None):
        if wait is not None:
            wait()
        col = pl.multiple_of(c * C, C)
        sk = [skT_ref[pl.ds(i, 1), pl.ds(col, C)].astype(F32) for i in range(4)]
        dvec = d_s[:, pl.ds(col, C)]
        sl = (c & 1)
        yield from b_first(k_s.at[sl], v_s.at[sl], h_s.at[sl], sk, dvec, ht_s, xs, hs, f_ref, ax, ah, part)

    def gen_m():
        return b_mid(ax, ah, vs)

    def gen_k(c, blocks=range(4)):
        return b_back(vs, finv_ref, q_s.at[(c & 1)], o_s, blocks)

    def a1(s):
        return a_phase1(x_s, w_s, pl.multiple_of(s * (R // 2), R // 2), p_acc, z_acc, pb_s)

    def a2(s, slot, part=None):
        return a_phase2(x_s, w_s, pl.multiple_of(s * (R // 2), R // 2), zt_s, m_s, wg_s, oa_s.at[slot], part)

    def oa_half_cp(hf):
        return pltpu.make_async_copy(oa_s.bitcast(BF).at[1, pl.ds(MA * hf, MA), :],
                                     o_hbm.at[0, pl.ds(S - R + MA * hf, MA), pl.ds(0, D)], sem_ob.at[1 + hf])

    def post_f(c):
        @pl.when(c + 1 < NT)
        def _():
            q_cp(c + 1).start()

        @pl.when(c + 2 < NT)
        def _():
            for cp in f_in(c + 2):
                cp.start()

    def pre_kf(c):
        q_cp(c).wait()

        @pl.when(c + 1 < NT)
        def _():
            for cp in f_in(c + 1):
                cp.wait()

        @pl.when(c >= 1)
        def _():
            ob_cp(c - 1).wait()

    flag_s[0] = 1
    x_cp(0).start()
    wc_cp(0).start()
    wc_cp(1).start()
    for g in range(2, 8):
        wc_cp(g).start()
    for cp in c_cps[:3]:
        cp.start()
    for cp in f_in(0):
        cp.start()
    x_cp(1).start()
    c_cps[3].start()
    z_acc[...] = jnp.zeros_like(z_acc)
    p_acc[7] = jnp.zeros((128, D), F32)
    for sl in range(2):
        k_s[sl, pl.ds(0, 16), :] = jnp.zeros((16, C), BF)
    with jax.named_scope("w_x0"):
        x_cp(0).wait()

    def wait_chunk(g):
        for gg in S0_WAITS.get(g, ()):
            wc_cp(gg).wait()
        if g == S0_F_AT:
            for cp in c_cps[:3]:
                cp.wait()
            d_s[...] = d_ref[...].reshape(1, D).astype(F32)
            for cp in f_in(0):
                cp.wait()

    with jax.named_scope("s0"):
        _interleave(a_phase1(x_s, w_s, 0, p_acc, z_acc, pb_s, wait_chunk),
                    gen_f(0), A1_TOT, BF_TOT, lead=S0_F_AT / 8 + 0.01)
    x_cp(2).start()
    q_cp(0).start()
    for cp in f_in(1):
        cp.start()
    post_f(0)
    for i in range(3, NR):
        x_cp(i).start()
    wq_cp.start()
    wv_cp.start()
    wo_cp.start()

    def phase1_body(s, carry):
        c = (s - 1) >> 1
        x_cp(s).wait()

        @pl.when((s & 1) == 1)
        def _():
            with jax.named_scope("a1m"):
                _interleave(a1(s), gen_m(), A1_TOT, BM_TOT)

        @pl.when((s & 1) == 0)
        def _():
            pre_kf(c)

            @pl.when(s == 2)
            def _():
                c_cps[3].wait()

        @pl.when((s & 1) == 0)
        def _():
            with jax.named_scope("a1kf"):
                _interleave(a1(s), _chain(gen_k(c), gen_f(c + 1)), A1_TOT, BK_TOT + BF_TOT, tail=0.03)

        @pl.when(flag_s[0] + (s & 1) == 1)
        def _():
            ob_cp(c).start()
            post_f(c + 1)
        return carry

    lax.fori_loop(1, 8, phase1_body, 0)

    wq_cp.wait()
    wv_cp.wait()
    wo_cp.wait()
    pre_kf(3)
    @pl.when(flag_s[0] == 1)
    def _():
        with jax.named_scope("bd"):
            a_boundary_prep(z_acc, zt_s)
            last_p = _p_dots(p_acc, 7, _bf(pb_s[...]), _bf(x_s[pl.ds((S - R) // 2, R // 2), :]))
            _interleave(_chain(last_p, a_boundary(p_acc, w_s, wo_s, m_s)), _chain(gen_k(3), gen_f(4)),
                        BD_TOT + 512, BK_TOT + BF_TOT)

    ob_cp(3).start()
    post_f(4)

    def phase2_body(s, carry):
        c = 4 + (s >> 1)

        @pl.when(s >= 2)
        def _():
            oa_cp(s - 2, (s & 1)).wait()

        @pl.when((s & 1) == 0)
        def _():
            with jax.named_scope("a2m"):
                _interleave(a2(s, 0), gen_m(), A2_TOT, BM_TOT)

        @pl.when((s & 1) == 1)
        def _():
            pre_kf(c)

        @pl.when((s & 1) == 1)
        def _():
            with jax.named_scope("a2kf"):
                _interleave(a2(s, 1), _chain(gen_k(c), gen_f(c + 1)), A2_TOT, BK_TOT + BF_TOT)

        @pl.when(flag_s[0] + (s & 1) == 1)
        def _():
            oa_cp(s, 0).start()

        @pl.when(flag_s[0] + (s & 1) == 2)
        def _():
            oa_cp(s, 1).start()
            ob_cp(c).start()
            post_f(c + 1)
        return carry

    lax.fori_loop(0, 7, phase2_body, 0)
    oa_cp(5, 1).wait()
    pre_kf(7)

    @pl.when(flag_s[0] == 1)
    def _():
        with jax.named_scope("last"):
            _interleave(a2(7, 1, "head"), gen_k(NT - 1), A2_TOT - 8 * A2_WO, BK_TOT, tail=LAST_TAIL)
    ob_cp(7).start()
    oa_half_cp(0).start()

    @pl.when(flag_s[0] == 1)
    def _():
        with jax.named_scope("last2"):
            _run(a2(7, 1, "tail"))
    oa_half_cp(1).start()
    with jax.named_scope("endwait"):
        oa_cp(6, 0).wait()
        ob_cp(7).wait()
        oa_half_cp(0).wait()
        oa_half_cp(1).wait()


@jax.jit
def pallas_concat_heads__linear_attn_block__ssm_conv_h3__prompt_kernel(A_x, A_wqkv, A_wo, B_q, B_k, B_v, B_shift_k, B_ssm_k, B_ssm_D):
    any_spec = pl.BlockSpec(memory_space=pl.ANY)
    return pl.pallas_call(
        kernel,
        in_specs=[any_spec] * 11,
        out_specs=any_spec,
        out_shape=jax.ShapeDtypeStruct((1, S, 2 * D), BF),
        scratch_shapes=[
            pltpu.VMEM((S // 2, D), U32),
            pltpu.VMEM((D // 2, 3 * D), U32),
            pltpu.VMEM((D // 2, D), U32),
            pltpu.VMEM((D // 2, D), U32),
            pltpu.VMEM((8, 128, D), F32),
            pltpu.VMEM((8, D), F32),
            pltpu.VMEM((8, D), F32),
            pltpu.VMEM((R // MA, MA // 2, D), U32),
            pltpu.VMEM((2, R // 2, D), U32),
            pltpu.VMEM((2, S + 16, C), BF),
            pltpu.VMEM((2, S + 32, C), BF),
            pltpu.VMEM((2, S + 16, C), BF),
            pltpu.VMEM((2, C // 2, S), U32),
            pltpu.VMEM((S + 16, C), BF),
            pltpu.VMEM((S // 2 + 8, C), U32),
            pltpu.VMEM((4, 4, 64, 128), U32),
            pltpu.VMEM((4, 4, 64, 128), U32),
            pltpu.VMEM((4, 4, 256, 128), F32),
            pltpu.VMEM((4, 4, 256, 128), F32),
            pltpu.VMEM((4, 4, 128, 128), U32),
            pltpu.VMEM((1, D), F32),
            pltpu.VMEM((4, D), BF),
            pltpu.VMEM((D,), BF),
            pltpu.VMEM((4, 128, 128), U32),
            pltpu.VMEM((4, 64, 256), U32),
            pltpu.VMEM((64, R), U32),
            pltpu.SMEM((1,), jnp.int32),
            pltpu.SemaphoreType.DMA((NR,)),
            pltpu.SemaphoreType.DMA((3,)),
            pltpu.SemaphoreType.DMA((8,)),
            pltpu.SemaphoreType.DMA((4,)),
            pltpu.SemaphoreType.DMA((8,)),
            pltpu.SemaphoreType.DMA((5,)),
            pltpu.SemaphoreType.DMA((2,)),
        ],
        compiler_params=pltpu.CompilerParams(vmem_limit_bytes=100 * 1024 * 1024, disable_bounds_checks=True, disable_semaphore_checks=True),
        name="fused",
    )(A_x, A_wqkv, A_wo, B_q, B_k, B_v, B_ssm_k, B_shift_k.T, B_ssm_D,
      jnp.asarray(_F_PK), jnp.asarray(_FINV_PK))
```

```python
import numpy as np
import jax
import jax.numpy as jnp
from jax import lax
from jax.experimental import pallas as pl
from jax.experimental.pallas import tpu as pltpu

S, D = 2048, 1024
C = 128
NT = D // C
MF = 1024
R = 256
NR = S // R
MA = 128
BF = jnp.bfloat16
F32 = jnp.float32
U32 = jnp.uint32

A2_WQ = 256
A2_WO = 256
NORM_GROUP = 16
FWD_CH = 128
BACK_CH = 64


def _make_consts():
    p = np.arange(16)[:, None]
    s = np.arange(8)[None, :]
    k1 = np.where(p < 8, 2 * (8 * p + s), 2 * (8 * (p - 8) + s) + 1)
    t1 = np.arange(128)
    F = np.zeros((4, 256, 128), np.float64)
    for t2 in range(4):
        th = 2 * np.pi * (4 * t1[None, None, :] + t2) * (k1[:, :, None] + 0.5) / MF
        F[t2] = np.stack([np.cos(th), -np.sin(th)], axis=1).reshape(256, 128)
    Finv = np.transpose(F.reshape(4, 16, 2, 8, 128), (0, 4, 1, 3, 2)).reshape(4, 128, 256) * (2.0 / MF)
    c = np.arange(128)
    perm = 16 * (c // 16) + 8 * ((c & 1)) + (c % 16) // 2
    F = F[:, :, perm]
    return F.astype(np.float32), Finv.astype(np.float32)


def _pack_rows(a):
    a = np.ascontiguousarray(a, np.float32)
    u = a.view(np.uint32)
    b = ((u + 0x7FFF + ((u >> 16) & 1)) >> 16).astype(np.uint32)
    return (b[..., 0::2, :] | (b[..., 1::2, :] << 16)).astype(np.uint32)


_F_NP, _FINV_NP = _make_consts()
_F_PK = _pack_rows(_F_NP)
_FINV_PK = _pack_rows(_FINV_NP)


def _lo(w):
    return pltpu.bitcast(w << 16, F32)


def _hi(w):
    return pltpu.bitcast(w & jnp.uint32(0xFFFF0000), F32)


def _bf(w):
    return pltpu.bitcast(w, BF)


def _pk(v):
    return pltpu.bitcast(v.astype(BF), U32)


def _dot(a, b):
    return jnp.dot(a, b, preferred_element_type=F32)


def _phi(t):
    return jnp.where(t > 0, t + 1.0, jnp.exp(t)) + 1e-6


def _radix4(A):
    (r0, i0), (r1, i1), (r2, i2), (r3, i3) = A
    a0r, a0i = r0 + r2, i0 + i2
    a1r, a1i = r0 - r2, i0 - i2
    b0r, b0i = r1 + r3, i1 + i3
    b1r, b1i = r1 - r3, i1 - i3
    return [(a0r + b0r, a0i + b0i), (a1r + b1i, a1i - b1r),
            (a0r - b0r, a0i - b0i), (a1r - b1i, a1i + b1r)]


def _iradix4(W):
    (r0, i0), (r1, i1), (r2, i2), (r3, i3) = W
    c0r, c0i = r0 + r2, i0 + i2
    c1r, c1i = r0 - r2, i0 - i2
    d0r, d0i = r1 + r3, i1 + i3
    d1r, d1i = r1 - r3, i1 - i3
    return [(c0r + d0r, c0i + d0i), (c1r - d1i, c1i + d1r),
            (c0r - d0r, c0i - d0i), (c1r + d1i, c1i - d1r)]


def b_front_x(k_s, v_s, sk, xs, j):
    kw = k_s.bitcast(U32)
    vw = v_s.bitcast(U32)
    s0, s1, s2, s3 = sk
    for n in range(8):
        t0 = 128 * j + 16 * n
        base = 8 + 2 * t0
        E = kw[pl.ds(base, 16, stride=2), :]
        O = kw[pl.ds(base + 1, 16, stride=2), :]
        Ep = kw[pl.ds(base - 2, 16, stride=2), :]
        Op = kw[pl.ds(base - 1, 16, stride=2), :]
        k0, k1, k2, k3 = _lo(E), _hi(E), _lo(O), _hi(O)
        k1p, k2p, k3p = _hi(Ep), _lo(Op), _hi(Op)
        Ev = vw[pl.ds(2 * t0, 16, stride=2), :]
        Ov = vw[pl.ds(2 * t0 + 1, 16, stride=2), :]
        ks0 = s0 * k0 + s1 * k3p + s2 * k2p + s3 * k1p
        ks1 = s0 * k1 + s1 * k0 + s2 * k3p + s3 * k2p
        ks2 = s0 * k2 + s1 * k1 + s2 * k0 + s3 * k3p
        ks3 = s0 * k3 + s1 * k2 + s2 * k1 + s3 * k0
        kv = [ks0 * _lo(Ev), ks1 * _hi(Ev), ks2 * _lo(Ov), ks3 * _hi(Ov)]
        for t2 in range(4):
            xs[t2, j, pl.ds(8 * n, 8), :] = pltpu.pack_elementwise([kv[t2][0:8], kv[t2][8:16]], packed_dtype=BF)
        yield 100


def b_front_h(h_s, ht_s, hs, m):
    for tt in range(4):
        c0 = 512 * m + 128 * tt
        ht_s[pl.ds(c0 // 2, 64), :] = pltpu.bitcast(_bf(h_s[:, pl.ds(c0, 128)]).T, U32)
        yield 40
    hw = ht_s
    m16 = jnp.uint32(0xFFFF)
    mh = jnp.uint32(0xFFFF0000)
    for n in range(8):
        base = 256 * m + 32 * n
        A0 = hw[pl.ds(base + 0, 8, stride=2), :]
        B0 = hw[pl.ds(base + 16, 8, stride=2), :]
        A1 = hw[pl.ds(base + 1, 8, stride=2), :]
        B1 = hw[pl.ds(base + 17, 8, stride=2), :]
        P = [(A0 & m16) | (B0 << 16), (A0 >> 16) | (B0 & mh),
             (A1 & m16) | (B1 << 16), (A1 >> 16) | (B1 & mh)]
        for t2 in range(4):
            hs[t2, m, pl.ds(8 * n, 8), :] = P[t2]
        if n % 4 == 3:
            yield 48


def b_fwd(f_ref, xs, ax, j, dvec=None):
    CH = FWD_CH
    X = [_bf(xs[t2, j]) for t2 in range(4)]

    def finish(ch, A):
        for pp in range(CH // 16):
            p = ch * (CH // 16) + pp
            a = [(A[t2][16 * pp:16 * pp + 8], A[t2][16 * pp + 8:16 * pp + 16]) for t2 in range(4)]
            if dvec is not None:
                a[0] = (a[0][0] + dvec, a[0][1])
            Xk = _radix4(a)
            for k in range(4):
                ax[k, j, pl.ds(16 * p, 8), :] = Xk[k][0]
                ax[k, j, pl.ds(16 * p + 8, 8), :] = Xk[k][1]

    prev = None
    for ch in range(256 // CH):
        A = [_dot(_bf(f_ref[t2, pl.ds(ch * CH // 2, CH // 2), :]), X[t2]) for t2 in range(4)]
        if prev is not None:
            finish(*prev)
        prev = (ch, A)
        yield CH * 5
    finish(*prev)
    yield CH


def b_first(k_s, v_s, h_s, sk, dvec, ht_s, xs, hs, f_ref, ax, ah, part=None):
    fx = lambda j: b_front_x(k_s, v_s, sk, xs, j)
    fh = lambda m: b_front_h(h_s, ht_s, hs, m)
    dx = lambda j: b_fwd(f_ref, xs, ax, j)
    dh = lambda m: b_fwd(f_ref, hs, ah, m, dvec if m == 0 else None)
    if part == "x":
        seq = (fx(0), fx(1), dx(0), fx(2), dx(1), fx(3), dx(2), dx(3))
    elif part == "h":
        seq = (fh(0), fh(1), dh(0), fh(2), dh(1), fh(3), dh(2), dh(3))
    else:
        seq = (fx(0), fx(1), dx(0), fx(2), dx(1), fx(3), dx(2), fh(0), dx(3), fh(1),
               dh(0), fh(2), dh(1), fh(3), dh(2), dh(3))
    for g in seq:
        yield from g


BF_TOT = 32 * 100 + 4 * (160 + 96) + 8 * (256 * 5 + FWD_CH)


def b_mid(ax, ah, vs):
    for p in range(16):
        pos = p < 8
        r_re = pl.ds(16 * p, 8)
        r_im = pl.ds(16 * p + 8, 8)
        Zp = None
        for i in range(4):
            Z = []
            for k in range(4):
                wr = None
                wi = None
                for j in range(i + 1):
                    xr, xi = ax[k, j, r_re, :], ax[k, j, r_im, :]
                    gr, gi = ah[k, i - j, r_re, :], ah[k, i - j, r_im, :]
                    pr = xr * gr - xi * gi
                    pi = xr * gi + xi * gr
                    wr = pr if wr is None else wr + pr
                    wi = pi if wi is None else wi + pi
                Z.append((wr, wi))
            if Zp is None:
                W = Z
            elif pos:
                W = [(Z[k][0] - Zp[k][1], Z[k][1] + Zp[k][0]) for k in range(4)]
            else:
                W = [(Z[k][0] + Zp[k][1], Z[k][1] - Zp[k][0]) for k in range(4)]
            Zp = Z
            V = _iradix4(W)
            for t2 in range(4):
                vs[t2, i, pl.ds(8 * p, 8), :] = pltpu.pack_elementwise([V[t2][0], V[t2][1]], packed_dtype=BF)
            yield 40 + 32 * (i + 1) + (8 if i else 0)


def b_back(vs, finv_ref, q_s, o_s, blocks=range(4)):
    qw = q_s.bitcast(U32)
    ow = o_s.bitcast(U32)
    CH = BACK_CH

    def finish(base, y):
        E = qw[pl.ds(base, CH, stride=2), :]
        ow[pl.ds(base, CH, stride=2), :] = pltpu.pack_elementwise(
            [_lo(E) * y[0], _hi(E) * y[1]], packed_dtype=BF)

    prev = None
    for i in blocks:
        for hf in range(2):
            Vt = [_bf(vs[2 * hf + e, i]) for e in range(2)]
            for ch in range(128 // CH):
                y = [_dot(_bf(finv_ref[2 * hf + e, pl.ds(ch * CH // 2, CH // 2), :]), Vt[e]) for e in range(2)]
                if prev is not None:
                    finish(*prev)
                prev = (256 * i + 2 * CH * ch + hf, y)
                yield CH * 5
    finish(*prev)
    yield CH


def _p_dots(p_acc, g, pk, xt, first=False):
    pkt = pk.T
    for n in range(4):
        cs = pl.ds(256 * n, 256)
        d = _dot(pkt, xt[:, 256 * n:256 * (n + 1)])
        if first:
            p_acc[g, :, cs] = d
        else:
            p_acc[g, :, cs] += d
        yield 128


def _k_finish(z_acc, col, kf0, kf1):
    pk = jnp.concatenate([_phi(kf0), _phi(kf1)], axis=0)
    z_acc[:, pl.ds(col, 128)] += jnp.sum(pk.reshape(R // 8, 8, 128), axis=0)
    return pk.astype(BF)


def a_phase1(x_s, w_s, r0, p_acc, z_acc, pb_s, wait_chunk=None):
    rw = r0
    xprev = lambda: _bf(x_s[pl.ds(pl.multiple_of(rw - R // 2, R // 2), R // 2), :])
    xfull = lambda: _bf(x_s[pl.ds(rw, R // 2), :])
    pend = None
    pend2 = None
    first = wait_chunk is not None
    for g in range(8):
        if first:
            wait_chunk(g)
        wk = lambda: _bf(w_s[:, pl.ds(1024 + 128 * g, 128)])
        kf0 = _dot(_bf(x_s[pl.ds(rw, MA // 2), :]), wk())
        yield 256
        if g == 0 and not first:
            yield from _p_dots(p_acc, 7, _bf(pb_s[...]), xprev())
        if pend is not None:
            pend2 = (pend[0], _k_finish(z_acc, 128 * pend[0], pend[1], pend[2]))
        kf1 = _dot(_bf(x_s[pl.ds(pl.multiple_of(rw + MA // 2, MA // 2), MA // 2), :]), wk())
        yield 256
        if pend2 is not None:
            yield from _p_dots(p_acc, pend2[0], pend2[1], xfull(), first)
            pend2 = None
        pend = (g, kf0, kf1)
    pb_s[...] = pltpu.bitcast(_k_finish(z_acc, 128 * pend[0], pend[1], pend[2]), U32)
    yield 16


A1_TOT = 8 * 1024 + 16


def a_boundary_prep(z_acc, zt_s):
    z = jnp.sum(z_acc[...], axis=0, keepdims=True)
    zt_s[...] = jnp.broadcast_to(z, (8, D))


def a_boundary(p_acc, w_s, wo_s, m_s):
    ri = lax.broadcasted_iota(jnp.int32, (128, 128), 0) // 32
    ci = lax.broadcasted_iota(jnp.int32, (128, 128), 1) // 32
    same = ri == ci

    pb = [None] * 8
    kv = [None] * 8
    kvb = [None] * 8

    def prep(g):
        if g < 8:
            pb[g] = p_acc[g].astype(BF)

    def kv_dot(g):
        kv[g] = _dot(pb[g], _bf(w_s[:, pl.ds(2048 + 128 * g, 128)]))

    def mask(g):
        kvb[g] = jnp.where(same, kv[g], 0.0).astype(BF)

    def m_dots(g):
        m_s[pl.ds(64 * g, 64), :] = _pk(_dot(kvb[g], _bf(wo_s[pl.ds(64 * g, 64), :])))
        yield 256

    prep(0)
    prep(1)
    yield 32
    for t in range(10):
        if t < 8:
            kv_dot(t)
            prep(t + 2)
        if 1 <= t <= 8:
            mask(t - 1)
        if t < 8:
            yield 256
        if t >= 2:
            yield from m_dots(t - 2)


def _head_normalize_rows(rows, z):
    lane = lax.broadcasted_iota(jnp.int32, (8, 128), 1)
    cur = [r * z for r in rows]
    pos = [0] * len(cur)
    groups = [[j] for j in range(len(cur))]
    sh = 16
    while len(cur) > 1:
        nxt = []
        ng = []
        upper = (lane & sh) != 0
        for a in range(0, len(cur), 2):
            u = cur[a] + pltpu.roll(cur[a], sh, 1)
            v = cur[a + 1] + pltpu.roll(cur[a + 1], 128 - sh, 1)
            nxt.append(jnp.where(upper, u, v))
            for j in groups[a]:
                pos[j] |= sh
            ng.append(groups[a] + groups[a + 1])
        cur = nxt
        groups = ng
        sh //= 2
    m = cur[0]
    fill = 0
    while sh >= 1:
        m = m + pltpu.roll(m, sh, 1)
        fill |= sh
        sh //= 2
    r = pl.reciprocal(m + 1e-6, approx=True)
    return [rows[j] * jnp.take_along_axis(r, (lane & ~31) | (pos[j] | fill), axis=1) for j in range(len(rows))]


def _head_normalize(pq, z):
    rows = [pq[8 * j:8 * j + 8] for j in range(MA // 8)]
    out = []
    for a in range(0, len(rows), NORM_GROUP):
        out += _head_normalize_rows(rows[a:a + NORM_GROUP], z)
    return jnp.concatenate(out, axis=0)


def a_phase2(x_s, w_s, r0, zr_s, m_s, wg_s, oa_s, part=None):
    def fin(g, mc, qf):
        wg_s[mc, :, pl.ds(128 * g, 128)] = _pk(_head_normalize(_phi(qf), zr_s[:, pl.ds(128 * g, 128)]))

    def out_dot(mc, n):
        wg = _bf(wg_s[mc])
        oa_s[pl.ds(mc * (MA // 2), MA // 2), pl.ds(128 * n, 128)] = _pk(_dot(wg, _bf(m_s[:, pl.ds(128 * n, 128)])))

    p1 = None
    nmc = R // MA
    if part == "tail":
        for n in range(8):
            out_dot(nmc - 1, n)
            yield A2_WO
        return
    for mc in range(nmc):
        rw = pl.multiple_of(r0 + mc * (MA // 2), MA // 2)
        for g in range(8):
            xt = _bf(x_s[pl.ds(rw, MA // 2), :])
            qf = _dot(xt, _bf(w_s[:, pl.ds(128 * g, 128)]))
            if p1 is not None:
                fin(*p1)
            p1 = (g, mc, qf)
            yield A2_WQ
            if mc > 0 and g >= 3:
                out_dot(mc - 1, g - 3)
                yield A2_WO
    out_dot(nmc - 2, 5)
    fin(*p1)
    yield A2_WO
    out_dot(nmc - 2, 6)
    yield A2_WO
    out_dot(nmc - 2, 7)
    yield A2_WO
    if part == "head":
        return
    for n in range(8):
        out_dot(nmc - 1, n)
        yield A2_WO


A2_TOT = 16 * (A2_WQ + A2_WO)


def _interleave(a_items, b_items, a_tot, b_tot, lead=0.0, tail=0.0):
    a_done = 0.0
    b_done = 0.0
    a_alive = True
    b_alive = True
    while a_alive or b_alive:
        fa = (a_done / a_tot - lead) / (1.0 - lead - tail)
        fb = b_done / b_tot
        if b_alive and (not a_alive or fb < fa):
            try:
                b_done += next(b_items)
            except StopIteration:
                b_alive = False
        else:
            try:
                a_done += next(a_items)
            except StopIteration:
                a_alive = False


def _chain(*gens):
    for g in gens:
        yield from g


BFX_TOT = 32 * 100 + 4 * (256 * 5 + FWD_CH)
BM_TOT = 16 * (160 + 320 + 24)
BK_TOT = 8 * 128 * 5 + BACK_CH
S0_WAITS = {0: (0,), 1: (1, 2), 3: (3, 4, 5), 6: (6, 7)}
S0_F_AT = 6
LAST_TAIL = 0.1
BD_TOT = 8 * 512 + 32


def _when(cond):
    if isinstance(cond, bool):
        return (lambda f: f()) if cond else (lambda f: None)
    return pl.when(cond)


def _run(gen):
    for _ in gen:
        pass


def kernel(x_hbm, w_hbm, wo_hbm, q_hbm, k_hbm, v_hbm, h_hbm, skT_hbm, d_hbm, f_hbm, finv_hbm, o_hbm,
           x_s, w_s, wo_s, m_s, p_acc, z_acc, zt_s, wg_s, oa_s,
           q_s, k_s, v_s, h_s, o_s, ht_s, xs, hs, ax, ah, vs, d_s,
           skT_ref, d_ref, f_ref, finv_ref, pb_s, flag_s,
           sem_x, sem_w, sem_wc, sem_c, sem_b, sem_ob, sem_oa):
    def x_cp(i):
        return pltpu.make_async_copy(x_hbm.at[0, pl.ds(i * R, R), :],
                                     x_s.bitcast(BF).at[pl.ds(i * R, R), :], sem_x.at[i])

    def wc_cp(g):
        col = pl.multiple_of(1024 + 128 * g, 128)
        return pltpu.make_async_copy(w_hbm.at[:, pl.ds(col, 128)],
                                     w_s.bitcast(BF).at[:, pl.ds(col, 128)], sem_wc.at[g])

    wv_cp = pltpu.make_async_copy(w_hbm.at[:, pl.ds(2048, 1024)], w_s.bitcast(BF).at[:, pl.ds(2048, 1024)],
                                  sem_w.at[2])

    wq_cp = pltpu.make_async_copy(w_hbm.at[:, pl.ds(0, 1024)], w_s.bitcast(BF).at[:, pl.ds(0, 1024)], sem_w.at[0])
    wo_cp = pltpu.make_async_copy(wo_hbm, wo_s.bitcast(BF), sem_w.at[1])
    c_cps = [pltpu.make_async_copy(skT_hbm, skT_ref, sem_c.at[0]),
             pltpu.make_async_copy(d_hbm, d_ref, sem_c.at[1]),
             pltpu.make_async_copy(f_hbm, f_ref, sem_c.at[2]),
             pltpu.make_async_copy(finv_hbm, finv_ref, sem_c.at[3])]

    def f_in(c):
        col = pl.multiple_of(c * C, C)
        return [
            pltpu.make_async_copy(k_hbm.at[0, :, pl.ds(col, C)], k_s.at[(c & 1), pl.ds(16, S), :], sem_b.at[4 * ((c & 1)) + 0]),
            pltpu.make_async_copy(v_hbm.at[0, :, pl.ds(col, C)], v_s.at[(c & 1), pl.ds(0, S), :], sem_b.at[4 * ((c & 1)) + 1]),
            pltpu.make_async_copy(h_hbm.at[pl.ds(col, C), :], h_s.bitcast(BF).at[(c & 1)], sem_b.at[4 * ((c & 1)) + 2]),
        ]

    def q_cp(c):
        col = pl.multiple_of(c * C, C)
        return pltpu.make_async_copy(q_hbm.at[0, :, pl.ds(col, C)], q_s.at[(c & 1), pl.ds(0, S), :],
                                     sem_b.at[4 * ((c & 1)) + 3])

    def ob_cp(c):
        col = pl.multiple_of(D + c * C, C)
        return pltpu.make_async_copy(o_s.at[pl.ds(0, S), :], o_hbm.at[0, :, pl.ds(col, C)], sem_ob.at[0])

    def ob_last_cp(i):
        return pltpu.make_async_copy(o_s.at[pl.ds(512 * i, 512), :],
                                     o_hbm.at[0, pl.ds(512 * i, 512), pl.ds(D + (NT - 1) * C, C)], sem_ob.at[1 + i])

    def oa_cp(i, slot):
        r = pl.multiple_of(i * R, R)
        return pltpu.make_async_copy(oa_s.bitcast(BF).at[slot], o_hbm.at[0, pl.ds(r, R), pl.ds(0, D)], sem_oa.at[slot])

    def gen_f(c, wait=None, part=None):
        if wait is not None:
            wait()
        col = pl.multiple_of(c * C, C)
        sk = [skT_ref[pl.ds(i, 1), pl.ds(col, C)].astype(F32) for i in range(4)]
        dvec = d_s[:, pl.ds(col, C)]
        sl = (c & 1)
        yield from b_first(k_s.at[sl], v_s.at[sl], h_s.at[sl], sk, dvec, ht_s, xs, hs, f_ref, ax, ah, part)

    def gen_m():
        return b_mid(ax, ah, vs)

    def gen_k(c, blocks=range(4)):
        return b_back(vs, finv_ref, q_s.at[(c & 1)], o_s, blocks)

    def a1(s):
        return a_phase1(x_s, w_s, pl.multiple_of(s * (R // 2), R // 2), p_acc, z_acc, pb_s)

    def a2(s, slot, part=None):
        return a_phase2(x_s, w_s, pl.multiple_of(s * (R // 2), R // 2), zt_s, m_s, wg_s, oa_s.at[slot], part)

    def oa_half_cp(hf):
        return pltpu.make_async_copy(oa_s.bitcast(BF).at[1, pl.ds(MA * hf, MA), :],
                                     o_hbm.at[0, pl.ds(S - R + MA * hf, MA), pl.ds(0, D)], sem_ob.at[1 + hf])

    def post_f(c):
        @_when(c + 1 < NT)
        def _():
            q_cp(c + 1).start()

        @_when(c + 2 < NT)
        def _():
            for cp in f_in(c + 2):
                cp.start()

    def pre_kf(c):
        q_cp(c).wait()

        @_when(c + 1 < NT)
        def _():
            for cp in f_in(c + 1):
                cp.wait()

        @_when(c >= 1)
        def _():
            ob_cp(c - 1).wait()

    flag_s[0] = 1
    x_cp(0).start()
    wc_cp(0).start()
    wc_cp(1).start()
    for g in range(2, 8):
        wc_cp(g).start()
    for cp in c_cps[:3]:
        cp.start()
    for cp in f_in(0):
        cp.start()
    x_cp(1).start()
    c_cps[3].start()
    z_acc[...] = jnp.zeros_like(z_acc)
    p_acc[7] = jnp.zeros((128, D), F32)
    for sl in range(2):
        k_s[sl, pl.ds(0, 16), :] = jnp.zeros((16, C), BF)
    with jax.named_scope("w_x0"):
        x_cp(0).wait()

    def wait_chunk(g):
        for gg in S0_WAITS.get(g, ()):
            wc_cp(gg).wait()
        if g == S0_F_AT:
            for cp in c_cps[:3]:
                cp.wait()
            d_s[...] = d_ref[...].reshape(1, D).astype(F32)
            for cp in f_in(0):
                cp.wait()

    with jax.named_scope("s0"):
        _interleave(a_phase1(x_s, w_s, 0, p_acc, z_acc, pb_s, wait_chunk),
                    gen_f(0), A1_TOT, BF_TOT, lead=S0_F_AT / 8 + 0.01)
    x_cp(2).start()
    q_cp(0).start()
    for cp in f_in(1):
        cp.start()
    post_f(0)
    for i in range(3, NR):
        x_cp(i).start()
    wq_cp.start()
    wv_cp.start()
    wo_cp.start()

    def phase1_body(s, carry):
        c = (s - 1) >> 1
        x_cp(s).wait()

        @pl.when((s & 1) == 1)
        def _():
            with jax.named_scope("a1m"):
                _interleave(a1(s), gen_m(), A1_TOT, BM_TOT)

        @pl.when((s & 1) == 0)
        def _():
            pre_kf(c)

            @pl.when(s == 2)
            def _():
                c_cps[3].wait()

        @pl.when((s & 1) == 0)
        def _():
            with jax.named_scope("a1kf"):
                _interleave(a1(s), _chain(gen_k(c), gen_f(c + 1)), A1_TOT, BK_TOT + BF_TOT, tail=0.03)

        @pl.when(flag_s[0] + (s & 1) == 1)
        def _():
            ob_cp(c).start()
            post_f(c + 1)
        return carry

    lax.fori_loop(1, 8, phase1_body, 0)

    wq_cp.wait()
    wv_cp.wait()
    wo_cp.wait()
    pre_kf(3)
    @pl.when(flag_s[0] == 1)
    def _():
        with jax.named_scope("bd"):
            a_boundary_prep(z_acc, zt_s)
            last_p = _p_dots(p_acc, 7, _bf(pb_s[...]), _bf(x_s[pl.ds((S - R) // 2, R // 2), :]))
            _interleave(_chain(last_p, a_boundary(p_acc, w_s, wo_s, m_s)), _chain(gen_k(3), gen_f(4)),
                        BD_TOT + 512, BK_TOT + BF_TOT)

    ob_cp(3).start()
    post_f(4)

    def phase2_body(s, carry):
        c = 4 + (s >> 1)

        @pl.when(s >= 2)
        def _():
            oa_cp(s - 2, (s & 1)).wait()

        @pl.when((s & 1) == 0)
        def _():
            with jax.named_scope("a2m"):
                _interleave(a2(s, 0), gen_m(), A2_TOT, BM_TOT)

        @pl.when((s & 1) == 1)
        def _():
            pre_kf(c)

        @pl.when((s & 1) == 1)
        def _():
            with jax.named_scope("a2kf"):
                _interleave(a2(s, 1), _chain(gen_k(c), gen_f(c + 1)), A2_TOT, BK_TOT + BF_TOT)

        @pl.when(flag_s[0] + (s & 1) == 1)
        def _():
            oa_cp(s, 0).start()

        @pl.when(flag_s[0] + (s & 1) == 2)
        def _():
            oa_cp(s, 1).start()
            ob_cp(c).start()
            post_f(c + 1)
        return carry

    lax.fori_loop(0, 7, phase2_body, 0)
    oa_cp(5, 1).wait()
    pre_kf(7)

    @pl.when(flag_s[0] == 1)
    def _():
        with jax.named_scope("last"):
            _interleave(a2(7, 1, "head"), gen_k(NT - 1), A2_TOT - 8 * A2_WO, BK_TOT, tail=LAST_TAIL)
    ob_cp(7).start()
    oa_half_cp(0).start()

    @pl.when(flag_s[0] == 1)
    def _():
        with jax.named_scope("last2"):
            _run(a2(7, 1, "tail"))
    oa_half_cp(1).start()
    with jax.named_scope("endwait"):
        oa_cp(6, 0).wait()
        ob_cp(7).wait()
        oa_half_cp(0).wait()
        oa_half_cp(1).wait()


@jax.jit
def pallas_concat_heads__linear_attn_block__ssm_conv_h3__prompt_kernel(A_x, A_wqkv, A_wo, B_q, B_k, B_v, B_shift_k, B_ssm_k, B_ssm_D):
    any_spec = pl.BlockSpec(memory_space=pl.ANY)
    return pl.pallas_call(
        kernel,
        in_specs=[any_spec] * 11,
        out_specs=any_spec,
        out_shape=jax.ShapeDtypeStruct((1, S, 2 * D), BF),
        scratch_shapes=[
            pltpu.VMEM((S // 2, D), U32),
            pltpu.VMEM((D // 2, 3 * D), U32),
            pltpu.VMEM((D // 2, D), U32),
            pltpu.VMEM((D // 2, D), U32),
            pltpu.VMEM((8, 128, D), F32),
            pltpu.VMEM((8, D), F32),
            pltpu.VMEM((8, D), F32),
            pltpu.VMEM((R // MA, MA // 2, D), U32),
            pltpu.VMEM((2, R // 2, D), U32),
            pltpu.VMEM((2, S + 16, C), BF),
            pltpu.VMEM((2, S + 32, C), BF),
            pltpu.VMEM((2, S + 16, C), BF),
            pltpu.VMEM((2, C // 2, S), U32),
            pltpu.VMEM((S + 16, C), BF),
            pltpu.VMEM((S // 2 + 8, C), U32),
            pltpu.VMEM((4, 4, 64, 128), U32),
            pltpu.VMEM((4, 4, 64, 128), U32),
            pltpu.VMEM((4, 4, 256, 128), F32),
            pltpu.VMEM((4, 4, 256, 128), F32),
            pltpu.VMEM((4, 4, 128, 128), U32),
            pltpu.VMEM((1, D), F32),
            pltpu.VMEM((4, D), BF),
            pltpu.VMEM((D,), BF),
            pltpu.VMEM((4, 128, 128), U32),
            pltpu.VMEM((4, 64, 256), U32),
            pltpu.VMEM((R // 2, 128), U32),
            pltpu.SMEM((1,), jnp.int32),
            pltpu.SemaphoreType.DMA((NR,)),
            pltpu.SemaphoreType.DMA((3,)),
            pltpu.SemaphoreType.DMA((8,)),
            pltpu.SemaphoreType.DMA((4,)),
            pltpu.SemaphoreType.DMA((8,)),
            pltpu.SemaphoreType.DMA((5,)),
            pltpu.SemaphoreType.DMA((2,)),
        ],
        compiler_params=pltpu.CompilerParams(vmem_limit_bytes=100 * 1024 * 1024, disable_bounds_checks=True, disable_semaphore_checks=True),
        name="fused",
    )(A_x, A_wqkv, A_wo, B_q, B_k, B_v, B_ssm_k, B_shift_k.T, B_ssm_D,
      jnp.asarray(_F_PK), jnp.asarray(_FINV_PK))
```
